```python
import jax
import jax.numpy as jnp

def _softmax(x, axis=-1):
    return jax.nn.softmax(x, axis=axis)

def _gelu(x):
    return jax.nn.gelu(x, approximate=True)

def _silu(x):
    return jax.nn.silu(x)

def _sigmoid(x):
    return jax.nn.sigmoid(x)

def _layernorm(x, axis=-1, eps=1e-05):
    m = jnp.mean(x, axis=axis, keepdims=True)
    v = jnp.var(x, axis=axis, keepdims=True)
    return (x - m) / jnp.sqrt(v + eps)

def _scatter_add(tgt, idx, src, axis=0):
    return tgt.at[idx].add(src)

def _segment_sum(src, seg, n):
    return jax.ops.segment_sum(src, seg, n)

class _Rng:

    def __init__(self, key):
        self._k = key

    def _next(self):
        self._k, sub = jax.random.split(self._k)
        return sub

    def normal(self, shape):
        return jax.random.normal(self._next(), shape, dtype=jnp.bfloat16)

    def randint(self, lo, hi, shape):
        return jax.random.randint(self._next(), shape, lo, hi, dtype=jnp.int32)

    def uniform(self, shape, lo=0.0, hi=1.0):
        return jax.random.uniform(self._next(), shape, jnp.bfloat16, lo, hi)

    def permutation(self, n):
        return jax.random.permutation(self._next(), n)
kernel_name = 'concat_heads__spectral_gfnet__memory_aug_recurrent_mem_tr__prompt'

def setup_inputs():
    _rng = _Rng(jax.random.key(int.from_bytes(__import__("os").urandom(4), "little")))
    _w = lambda a: (lambda t: t.astype(jnp.bfloat16) if jnp.issubdtype(t.dtype, jnp.floating) else t)(jnp.asarray(a))

    def _A_setup():
        B, S, D = (1, 2048, 1024)
        Df = D // 2 + 1
        return {'x': _w((lambda *s: _rng.normal(s) * 0.05)(B, S, D)), 'w_r': _w((lambda *s: _rng.normal(s) * 0.05)(S, Df) * 0.02), 'w_i': _w((lambda *s: _rng.normal(s) * 0.05)(S, Df) * 0.02)}
    _A_in = _A_setup()

    def _B_setup():
        B, S, Dm = (1, 2048, 1024)
        H, Dh = (32, 128)
        M, seg = (8, 32)
        seg = min(seg, S)
        S = S // seg * seg
        return {'x': _w((lambda *s: _rng.normal(s) * 0.05)(B, S, Dm)), 'mem0': _w((lambda *s: _rng.normal(s) * 0.05)(B, M, Dm)), 'Wq': _w((lambda *s: _rng.normal(s) * 0.05)(Dm, H, Dh) * Dm ** (-0.5)), 'Wk': _w((lambda *s: _rng.normal(s) * 0.05)(Dm, H, Dh) * Dm ** (-0.5)), 'Wv': _w((lambda *s: _rng.normal(s) * 0.05)(Dm, H, Dh) * Dm ** (-0.5)), 'Wo': _w((lambda *s: _rng.normal(s) * 0.05)(H, Dh, Dm) * (H * Dh) ** (-0.5)), 'seg_len': seg}
    _B_in = _B_setup()
    return {'A_x': _A_in['x'], 'A_w_r': _A_in['w_r'], 'A_w_i': _A_in['w_i'], 'B_x': _B_in['x'], 'B_mem0': _B_in['mem0'], 'B_Wq': _B_in['Wq'], 'B_Wk': _B_in['Wk'], 'B_Wv': _B_in['Wv'], 'B_Wo': _B_in['Wo'], 'B_seg_len': _B_in['seg_len']}

def reference(A_x, A_w_r, A_w_i, B_x, B_mem0, B_Wq, B_Wk, B_Wv, B_Wo, B_seg_len):

    def _A_ref(x, w_r, w_i):
        B, S, D = x.shape
        X = (lambda x, axes=(-2, -1): jnp.fft.rfft2(x.astype(jnp.float32), axes=axes))(x, axes=(-2, -1))
        W = w_r + 1j * w_i
        X = X * W
        y = (lambda x, s, axes=(-2, -1): jnp.fft.irfft2(x, s=s, axes=axes).astype(jnp.bfloat16))(X, (S, D), axes=(-2, -1))
        return y

    def _B_ref(x, mem0, Wq, Wk, Wv, Wo, seg_len):
        B, S, Dm = x.shape
        H, Dh = (Wq.shape[1], Wq.shape[2])
        M = mem0.shape[1]
        scale = Dh ** (-0.5)
        n_seg = S // seg_len
        L = M + seg_len
        idx = jnp.arange(L)
        mask = (idx[:, None] < M) | (idx[:, None] >= idx[None, :])
        mem = mem0
        outs = []
        for s in range(n_seg):
            xs = x[:, s * seg_len:(s + 1) * seg_len, :].copy()
            h = jnp.concatenate([mem, xs], axis=1)
            q = jnp.einsum('btd,dhe->bhte', h, Wq)
            k = jnp.einsum('btd,dhe->bhte', h, Wk)
            v = jnp.einsum('btd,dhe->bhte', h, Wv)
            scores = jnp.einsum('bhqe,bhke->bhqk', q, k) * scale
            scores = jnp.where(mask[None, None], scores, -1000000000.0)
            p = _softmax(scores, axis=-1)
            o = jnp.einsum('bhqk,bhke->bhqe', p, v)
            o = jnp.einsum('bhte,hed->btd', o, Wo)
            mem = o[:, :M, :].copy()
            outs.append(o[:, M:, :])
        return jnp.concatenate(outs, axis=1)
    a = _A_ref(A_x, A_w_r, A_w_i)
    b = _B_ref(B_x, B_mem0, B_Wq, B_Wk, B_Wv, B_Wo, B_seg_len)
    return jnp.concatenate([a, b], axis=-1)
```

```python
import jax
import jax.numpy as jnp
import numpy as np
from jax import lax
import jax.experimental.pallas as pl
import jax.experimental.pallas.tpu as pltpu

f32, bf16, u32 = jnp.float32, jnp.bfloat16, jnp.uint32

S = 2048
D = 1024
H, DH = 32, 128
M = 8
SEG = 32
L = M + SEG
NSEG = S // SEG
GH = 4
NG = H // GH
RH = float(np.sqrt(0.5))


def _dft_constants():
    lane = np.arange(128)
    j = np.arange(64)

    def cs(r):
        th = 2 * np.pi * (((r + 8 * j)[:, None] * lane[None, :]) % D) / D
        return np.cos(th), -np.sin(th)

    c, s = cs(0)
    s[0] = np.cos(np.pi * lane)
    tiles = [np.concatenate([c, s])]
    c, s = cs(4)
    tiles.append(np.concatenate([c, s]))
    for r in (1, 2, 3):
        c, s = cs(r)
        c_, s_ = cs(8 - r)
        tiles += [np.concatenate([c, s]), np.concatenate([-s, c]),
                  np.concatenate([c_, s_]), np.concatenate([s_, -c_])]
    g = np.stack(tiles) * 2.0 ** -10
    mm = []
    for n1 in range(16):
        th = 2 * np.pi * (((n1 + 16 * lane)[:, None] * lane[None, :]) % S) / S
        mm.append(np.stack([np.cos(th), -np.sin(th)]))
    return g.astype(bf16), np.stack(mm).astype(bf16)


_G_CONST, _MM_CONST = _dft_constants()


def _dot(a, b):
    return lax.dot_general(a, b, (((1,), (0,)), ((), ())), preferred_element_type=f32)


def _dot_t(a, b):
    return lax.dot_general(a, b, (((1,), (1,)), ((), ())), preferred_element_type=f32)


def _lo_f32(w):
    return pltpu.bitcast(w << 16, f32)


def _hi_f32(w):
    return pltpu.bitcast(w & u32(0xFFFF0000), f32)


def _fft4(a, b, c, d, sgn):
    t0 = (a[0] + c[0], a[1] + c[1])
    t1 = (a[0] - c[0], a[1] - c[1])
    t2 = (b[0] + d[0], b[1] + d[1])
    t3 = (b[0] - d[0], b[1] - d[1])
    o0 = (t0[0] + t2[0], t0[1] + t2[1])
    o2 = (t0[0] - t2[0], t0[1] - t2[1])
    p = (t1[0] + t3[1], t1[1] - t3[0])
    m = (t1[0] - t3[1], t1[1] + t3[0])
    return (o0, p, o2, m) if sgn < 0 else (o0, m, o2, p)


def _fft16(x, sgn):
    y = [_fft4(x[a], x[a + 4], x[a + 8], x[a + 12], sgn) for a in range(4)]
    out = [None] * 16
    for kl in range(4):
        z = []
        for a in range(4):
            e = a * kl
            re, im = y[a][kl]
            if e == 0:
                v = (re, im)
            elif e == 4:
                v = (im, -re) if sgn < 0 else (-im, re)
            elif e == 2:
                v = ((re + im) * RH, (im - re) * RH) if sgn < 0 else ((re - im) * RH, (im + re) * RH)
            elif e == 6:
                v = ((im - re) * RH, (re + im) * -RH) if sgn < 0 else ((re + im) * -RH, (re - im) * RH)
            else:
                c, s = float(np.cos(np.pi * e / 8)), float(sgn * np.sin(np.pi * e / 8))
                v = (re * c - im * s, re * s + im * c)
            z.append(v)
        o = _fft4(*z, sgn)
        for kh in range(4):
            out[kl + 4 * kh] = o[kh]
    return out


def _spectral_forward(xa, g, mm, fr, fi, row0):
    def pair(jp, _):
        w = [jnp.concatenate([xa[t, pl.ds(jp + 64 * b, 8, stride=8), :] for b in range(16)], axis=0)
             for t in range(8)]
        for half, cvt in enumerate((_lo_f32, _hi_f32)):
            n1 = 2 * jp + half
            x = [cvt(v) for v in w]
            a = [x[i] + x[i + 4] for i in range(4)]
            b = [x[i] - x[i + 4] for i in range(4)]
            e0, e1 = a[0] + a[2], a[1] + a[3]
            t0, t1 = (b[1] - b[3]) * RH, (b[1] + b[3]) * RH
            pq = {1: (b[0] + t0, -b[2] - t1), 2: (a[0] - a[2], a[3] - a[1]), 3: (b[0] - t0, b[2] - t1)}
            dc = {0: _dot_t(g[0], (e0 + e1).astype(bf16)), 4: _dot_t(g[1], (e0 - e1).astype(bf16))}
            for r in (1, 2, 3):
                o = 2 + 4 * (r - 1)
                both = (_dot_t(jnp.concatenate([g[o], g[o + 2]], axis=0), pq[r][0].astype(bf16))
                        + _dot_t(jnp.concatenate([g[o + 1], g[o + 3]], axis=0), pq[r][1].astype(bf16)))
                dc[r], dc[8 - r] = both[:128], both[128:]
            dall = jnp.concatenate([dc[c] for c in range(8)], axis=0)
            er, ei = _dot(dall, mm[n1, 0]), _dot(dall, mm[n1, 1])
            for c in range(8):
                tr, ti = er[c * 128:c * 128 + 64], ei[c * 128:c * 128 + 64]
                br, bi = er[c * 128 + 64:c * 128 + 128], ei[c * 128 + 64:c * 128 + 128]
                if c == 0:
                    fr[n1, 512:520, :] = br[:8]
                    fi[n1, 512:520, :] = bi[:8]
                    br = jnp.concatenate([jnp.where(row0, 0.0, br[:8]), br[8:]], axis=0)
                    bi = jnp.concatenate([jnp.where(row0, 0.0, bi[:8]), bi[8:]], axis=0)
                fr[n1, c * 64:(c + 1) * 64, :] = tr - bi
                fi[n1, c * 64:(c + 1) * 64, :] = ti + br
        return 0

    lax.fori_loop(0, 8, pair, 0)


def _spectral_filter(wra, wia, wr_ny, wi_ny, fr, fi, row0):
    def block(r0, wr, wi):
        z = _fft16([(fr[n, pl.ds(r0, 8), :], fi[n, pl.ds(r0, 8), :]) for n in range(16)], -1)
        z = [(z[k][0] * wr[k] - z[k][1] * wi[k], z[k][0] * wi[k] + z[k][1] * wr[k]) for k in range(16)]
        z = _fft16(z, 1)
        for n in range(16):
            fr[n, pl.ds(r0, 8), :] = z[n][0]
            fi[n, pl.ds(r0, 8), :] = z[n][1]

    half_dc = jnp.where(row0, 0.5, 1.0)

    def two_blocks(i, _):
        rho, jb = i // 8, i % 8
        sc = jnp.where(i == 0, half_dc, 1.0)
        wr = [wra[k, pl.ds(rho + 32 * jb, 8, stride=4), :] for k in range(16)]
        wi = [wia[k, pl.ds(rho + 32 * jb, 8, stride=4), :] for k in range(16)]
        r0 = pl.multiple_of(rho * 128 + jb * 8, 8)
        block(r0, [_lo_f32(v) * sc for v in wr], [_lo_f32(v) * sc for v in wi])
        block(r0 + 64, [_hi_f32(v) for v in wr], [_hi_f32(v) for v in wi])
        return 0

    lax.fori_loop(0, 32, two_blocks, 0)
    nr = wr_ny[0:1, :].astype(f32) * 0.5
    ni = wi_ny[0:1, :].astype(f32) * 0.5
    block(512, [nr[:, k * 128:(k + 1) * 128] for k in range(16)],
          [ni[:, k * 128:(k + 1) * 128] for k in range(16)])


def _spectral_inverse(fr, fi, g, mm, ya, row0):
    def pair(jp, _):
        ys = []
        for half in range(2):
            n1 = 2 * jp + half
            m2 = jnp.concatenate([mm[n1, 0], mm[n1, 1]], axis=1)
            tc = []
            for c in range(8):
                br, bi = fr[n1, c * 64:(c + 1) * 64, :], fi[n1, c * 64:(c + 1) * 64, :]
                b1, b2 = bi, -br
                if c == 0:
                    b1 = jnp.concatenate([jnp.where(row0, fr[n1, 512:520, :], b1[:8]), b1[8:]], axis=0)
                    b2 = jnp.concatenate([jnp.where(row0, fi[n1, 512:520, :], b2[:8]), b2[8:]], axis=0)
                rhs = jnp.concatenate([jnp.concatenate([br, b1], axis=0),
                                       jnp.concatenate([bi, b2], axis=0)], axis=1).astype(bf16)
                tc.append(_dot_t(m2, rhs))
            v0, v4 = _dot(tc[0], g[0]), _dot(tc[4], g[1])
            pq = []
            for r in (1, 2, 3):
                o = 2 + 4 * (r - 1)
                pq.append((_dot(tc[r], g[o]) + _dot(tc[8 - r], g[o + 2]),
                           _dot(tc[r], g[o + 1]) + _dot(tc[8 - r], g[o + 3])))
            (p1, q1), (p2, q2), (p3, q3) = pq
            e0, e1 = v0 + v4, v0 - v4
            a0, a2, a1, a3 = e0 + p2, e0 - p2, e1 - q2, e1 + q2
            b0, b2 = p1 + p3, q3 - q1
            t0, t1 = p1 - p3, q1 + q3
            b1, b3 = (t0 - t1) * RH, (t0 + t1) * -RH
            ys.append([a0 + b0, a1 + b1, a2 + b2, a3 + b3, a0 - b0, a1 - b1, a2 - b2, a3 - b3])
        for t in range(8):
            lo = pltpu.bitcast(ys[0][t].astype(bf16).astype(f32), u32) >> 16
            hi = pltpu.bitcast(ys[1][t].astype(bf16).astype(f32), u32)
            w = lo | hi
            for b in range(16):
                ya[t, pl.ds(jp + 64 * b, 8, stride=8), :] = w[b * 8:(b + 1) * 8]
        return 0

    lax.fori_loop(0, 8, pair, 0)


def _repack_head_pair(w, j):
    def body(i, _):
        for t in range(8):
            r0 = pl.multiple_of(i * 128 + t * 16, 16)
            even = w[j, pl.ds(r0, 8, stride=2), :]
            odd = w[j, pl.ds(r0 + 1, 8, stride=2), :]
            w[j, pl.ds(r0, 8), :] = (even & u32(0xFFFF)) | (odd << 16)
            w[j, pl.ds(r0 + 8, 8), :] = (even >> 16) | (odd & u32(0xFFFF0000))
        return 0

    lax.fori_loop(0, 8, body, 0)


def _head_weight(w, h):
    packed = w[h // 2].reshape(64, 2, 8, 128)[:, h % 2].reshape(512, 128)
    return pltpu.bitcast(packed, bf16)


def _segment(s, mem, xb, wq, wk, wv, wo, ob, mask):
    r0 = pl.multiple_of(s * SEG, SEG)
    hh = jnp.concatenate([mem, xb[pl.ds(r0, SEG), :].astype(f32)], axis=0)
    q, k, v, p, o = {}, {}, {}, {}, {}
    acc = [None] * 8
    heads = lambda grp: range(grp * GH, (grp + 1) * GH)

    def project(grp):
        for h in heads(grp):
            q[h] = _dot(hh, _head_weight(wq, h))
            k[h] = _dot(hh, _head_weight(wk, h)).astype(bf16)
            v[h] = _dot(hh, _head_weight(wv, h)).astype(bf16)

    def softmax(grp):
        for h in heads(grp):
            sc = jnp.where(mask, _dot_t(q.pop(h), k.pop(h)) * DH ** -0.5, -1e9)
            e = jnp.exp(sc - jnp.max(sc, axis=1, keepdims=True))
            p[h] = e / jnp.sum(e, axis=1, keepdims=True)

    def mix(grp):
        for h in heads(grp):
            o[h] = _dot(p.pop(h), v.pop(h))

    def out_project(grp):
        og = jnp.concatenate([o.pop(h) for h in heads(grp)], axis=1)
        for j in range(8):
            t = _dot(og, pltpu.bitcast(wo[j, pl.ds(grp * GH * DH // 2, GH * DH // 2), :], bf16))
            acc[j] = t if acc[j] is None else acc[j] + t

    for t in range(NG + 3):
        if t < NG:
            project(t)
        if 0 <= t - 1 < NG:
            softmax(t - 1)
        if 0 <= t - 2 < NG:
            mix(t - 2)
        if 0 <= t - 3 < NG:
            out_project(t - 3)
    res = jnp.concatenate(acc, axis=1)
    ob[pl.ds(r0, SEG), :] = res[M:].astype(bf16)
    return res[:M].astype(bf16).astype(f32)


def _kernel(ax_hbm, wr_hbm, wi_hbm, wr_ny, wi_ny, g_hbm, mm_hbm,
            bx_hbm, m0_hbm, wq_hbm, wk_hbm, wv_hbm, wo_hbm, out_hbm,
            xa, wra, wia, g, mm, fr, fi, ya,
            wq, wk, wv, wo, xb, m0, ob, sems, ya_sem, ob_sem):
    n_sem = [0]

    def copy(src, dst):
        n_sem[0] += 1
        return pltpu.make_async_copy(src, dst, sems.at[n_sem[0] - 1])

    def lane_tile(ref, t):
        return ref.at[:, pl.ds(t * 128, 128)]

    c_ax = [copy(g_hbm, g), copy(mm_hbm, mm)]
    c_ax += [copy(lane_tile(ax_hbm.bitcast(u32), t), xa.at[t]) for t in range(8)]
    c_aw = [copy(lane_tile(src.at[pl.ds(0, 512), :].bitcast(u32), t), dst.at[t])
            for src, dst in ((wr_hbm, wra), (wi_hbm, wia)) for t in range(16)]
    c_qkv = [[copy(src.bitcast(u32).at[:, j, :], dst.at[j]) for j in range(H // 2)]
             for src, dst in ((wq_hbm, wq), (wk_hbm, wk), (wv_hbm, wv))]
    c_rest = [copy(lane_tile(wo_hbm.bitcast(u32), t), wo.at[t]) for t in range(8)]
    c_rest += [copy(m0_hbm, m0), copy(bx_hbm, xb)]
    for c in c_ax + c_aw + sum(c_qkv, []) + c_rest:
        c.start()

    row0 = lax.broadcasted_iota(jnp.int32, (8, 128), 0) == 0
    for c in c_ax:
        c.wait()
    _spectral_forward(xa, g, mm, fr, fi, row0)
    for c in c_aw:
        c.wait()
    _spectral_filter(wra, wia, wr_ny, wi_ny, fr, fi, row0)
    _spectral_inverse(fr, fi, g, mm, ya, row0)
    c_ya = [pltpu.make_async_copy(ya.at[t], lane_tile(out_hbm.bitcast(u32), t), ya_sem) for t in range(8)]
    for c in c_ya:
        c.start()

    for w, copies in zip((wq, wk, wv), c_qkv):
        for j, c in enumerate(copies):
            c.wait()
            _repack_head_pair(w, j)
    for c in c_rest:
        c.wait()

    row = lax.broadcasted_iota(jnp.int32, (L, L), 0)
    col = lax.broadcasted_iota(jnp.int32, (L, L), 1)
    mask = (row < M) | (row >= col)

    def step(s, mem):
        mem = _segment(s, mem, xb, wq, wk, wv, wo, ob, mask)
        r0 = pl.multiple_of(s * SEG, SEG)
        pltpu.make_async_copy(ob.at[pl.ds(r0, SEG)], out_hbm.at[pl.ds(r0, SEG), pl.ds(D, D)], ob_sem).start()
        return mem

    lax.fori_loop(0, NSEG, step, m0[...].astype(f32))
    for c in c_ya:
        c.wait()
    pltpu.make_async_copy(ob, ob, ob_sem).wait()


def _run(A_x, A_w_r, A_w_i, B_x, B_mem0, B_Wq, B_Wk, B_Wv, B_Wo):
    hbm = pl.BlockSpec(memory_space=pltpu.HBM)
    nyquist = pl.BlockSpec((8, S), lambda i: (D // 16, 0))
    out = pl.pallas_call(
        _kernel,
        out_shape=jax.ShapeDtypeStruct((S, 2 * D), bf16),
        grid=(1,),
        in_specs=[hbm, hbm, hbm, nyquist, nyquist] + [hbm] * 8,
        out_specs=hbm,
        scratch_shapes=[
            pltpu.VMEM((8, S // 2, 128), u32),
            pltpu.VMEM((16, 256, 128), u32),
            pltpu.VMEM((16, 256, 128), u32),
            pltpu.VMEM((14, 128, 128), bf16),
            pltpu.VMEM((16, 2, 128, 128), bf16),
            pltpu.VMEM((16, 520, 128), f32),
            pltpu.VMEM((16, 520, 128), f32),
            pltpu.VMEM((8, S // 2, 128), u32),
            pltpu.VMEM((H // 2, D, 128), u32),
            pltpu.VMEM((H // 2, D, 128), u32),
            pltpu.VMEM((H // 2, D, 128), u32),
            pltpu.VMEM((8, H * DH // 2, 128), u32),
            pltpu.VMEM((S, D), bf16),
            pltpu.VMEM((M, D), bf16),
            pltpu.VMEM((S, D), bf16),
            pltpu.SemaphoreType.DMA((100,)),
            pltpu.SemaphoreType.DMA(()),
            pltpu.SemaphoreType.DMA(()),
        ],
        compiler_params=pltpu.CompilerParams(
            dimension_semantics=("arbitrary",), vmem_limit_bytes=110 * 1024 * 1024),
        name="gfnet_rmt",
    )(A_x.reshape(S, D), A_w_r.T, A_w_i.T, A_w_r.T, A_w_i.T, _G_CONST, _MM_CONST,
      B_x.reshape(S, D), B_mem0.reshape(M, D), B_Wq, B_Wk, B_Wv, B_Wo.reshape(H * DH, D))
    return out.reshape(1, S, 2 * D)


_run_jit = jax.jit(_run)


def pallas_concat_heads__spectral_gfnet__memory_aug_recurrent_mem_tr__prompt_kernel(
    A_x, A_w_r, A_w_i, B_x, B_mem0, B_Wq, B_Wk, B_Wv, B_Wo, B_seg_len,
):
    assert A_x.shape == (1, S, D) and B_x.shape == (1, S, D) and B_mem0.shape == (1, M, D)
    assert B_Wq.shape == (D, H, DH) and B_Wo.shape == (H, DH, D)
    assert B_seg_len == SEG, "the kernel is specialised to the problem's segment length"
    return _run_jit(A_x, A_w_r, A_w_i, B_x, B_mem0, B_Wq, B_Wk, B_Wv, B_Wo)
```

```python
import functools

import jax
import jax.numpy as jnp
import numpy as np
from jax import lax
import jax.experimental.pallas as pl
import jax.experimental.pallas.tpu as pltpu

f32, bf16, u32 = jnp.float32, jnp.bfloat16, jnp.uint32

S = 2048
D = 1024
H, DH = 32, 128
M = 8
SEG = 32
L = M + SEG
NSEG = S // SEG
GH = 4
NG = H // GH
RH = float(np.sqrt(0.5))
EARLY = 8
FWD_GROUPS = ((1,), (2, 3), (4, 5, 6, 7))
N_STEPS = NSEG
PAIRS_PER_ITER = 4
FILTER_AT = 2
UNROLL = 2
BF_ROWS = 128
SPLIT_HEADS = 0
SCHED = 2
SOFTMAX = 2
FILTER_MODE = 2
PACE_FROM = 2
LOG2E = float(np.log2(np.e))
FLAGS = None
LHS_DTYPE = bf16


def _row_pair_words(a):
    bits = a.astype(bf16).view(np.uint16).astype(np.uint32)
    return bits[..., 0::2, :] | (bits[..., 1::2, :] << 16)


def _dft_constants():
    lane = np.arange(128)
    j = np.arange(64)

    def cs(r):
        th = 2 * np.pi * (((r + 8 * j)[:, None] * lane[None, :]) % D) / D
        return np.cos(th), -np.sin(th)

    c, s = cs(0)
    s[0] = np.cos(np.pi * lane)
    tiles = [np.concatenate([c, s])]
    c, s = cs(4)
    tiles.append(np.concatenate([c, s]))
    for r in (1, 2, 3):
        c, s = cs(r)
        c_, s_ = cs(8 - r)
        tiles += [np.concatenate([c, s]), np.concatenate([-s, c]),
                  np.concatenate([c_, s_]), np.concatenate([s_, -c_])]
    g = np.stack(tiles) * 2.0 ** -10
    mm = []
    for n1 in range(16):
        th = 2 * np.pi * (((n1 + 16 * lane)[:, None] * lane[None, :]) % S) / S
        mm.append(np.stack([np.cos(th), -np.sin(th)]))
    return _row_pair_words(g), _row_pair_words(np.stack(mm).reshape(32, 128, 128))


_G_CONST, _MM_CONST = _dft_constants()


def _dot(a, b):
    return lax.dot_general(a, b, (((1,), (0,)), ((), ())), preferred_element_type=f32)


def _dot_t(a, b):
    return lax.dot_general(a, b, (((1,), (1,)), ((), ())), preferred_element_type=f32)


def _lo_f32(w):
    return pltpu.bitcast(w << 16, f32)


def _hi_f32(w):
    return pltpu.bitcast(w & u32(0xFFFF0000), f32)


def _every_other_tile(words, parity):
    n = words.shape[0] // 16
    return pltpu.bitcast(words.reshape(n, 2, 8, 128)[:, parity].reshape(n * 8, 128), bf16)


def _fft4(a, b, c, d, sgn):
    t0 = (a[0] + c[0], a[1] + c[1])
    t1 = (a[0] - c[0], a[1] - c[1])
    t2 = (b[0] + d[0], b[1] + d[1])
    t3 = (b[0] - d[0], b[1] - d[1])
    o0 = (t0[0] + t2[0], t0[1] + t2[1])
    o2 = (t0[0] - t2[0], t0[1] - t2[1])
    p = (t1[0] + t3[1], t1[1] - t3[0])
    m = (t1[0] - t3[1], t1[1] + t3[0])
    return (o0, p, o2, m) if sgn < 0 else (o0, m, o2, p)


def _fft16(x, sgn):
    y = [_fft4(x[a], x[a + 4], x[a + 8], x[a + 12], sgn) for a in range(4)]
    out = [None] * 16
    for kl in range(4):
        z = []
        for a in range(4):
            e = a * kl
            re, im = y[a][kl]
            if e == 0:
                v = (re, im)
            elif e == 4:
                v = (im, -re) if sgn < 0 else (-im, re)
            elif e == 2:
                v = ((re + im) * RH, (im - re) * RH) if sgn < 0 else ((re - im) * RH, (im + re) * RH)
            elif e == 6:
                v = ((im - re) * RH, (re + im) * -RH) if sgn < 0 else ((re + im) * -RH, (re - im) * RH)
            else:
                c, s = float(np.cos(np.pi * e / 8)), float(sgn * np.sin(np.pi * e / 8))
                v = (re * c - im * s, re * s + im * c)
            z.append(v)
        o = _fft4(*z, sgn)
        for kh in range(4):
            out[kl + 4 * kh] = o[kh]
    return out


def _forward_butterflies(jp, xa):
    def rows(r0, cvt):
        x = [cvt(xa[jp, pl.ds(r0, 8), pl.ds(t * 128, 128)]) for t in range(8)]
        a = [x[i] + x[i + 4] for i in range(4)]
        b = [x[i] - x[i + 4] for i in range(4)]
        e0, e1 = a[0] + a[2], a[1] + a[3]
        t0, t1 = (b[1] - b[3]) * RH, (b[1] + b[3]) * -RH
        return [e0 + e1, e0 - e1, b[0] + t0, t1 - b[2], a[0] - a[2], a[3] - a[1], b[0] - t0, b[2] + t1]

    us = []
    for cvt in (_lo_f32, _hi_f32):
        chunks = []
        for r0 in range(0, 128, BF_ROWS):
            parts = [rows(r, cvt) for r in range(r0, r0 + BF_ROWS, 8)]
            chunks.append([jnp.concatenate([p[t] for p in parts], axis=0).astype(bf16) for t in range(8)])
        us.append([jnp.concatenate([c[t] for c in chunks], axis=0) for t in range(8)])
    return us


def _forward_matmuls(jp, us, g, mm, fr, fi, row0):
    dcs = []
    for u in us:
        dc = {0: _dot_t(g(0), u[0]), 4: _dot_t(g(1), u[1])}
        for r in (1, 2, 3):
            o = 2 + 4 * (r - 1)
            p, q = u[2 * r], u[2 * r + 1]
            dc[r] = _dot_t(g(o), p) + _dot_t(g(o + 1), q)
            dc[8 - r] = _dot_t(g(o + 2), p) + _dot_t(g(o + 3), q)
        dcs.append(dc)
    for half, dc in enumerate(dcs):
        n1 = 2 * jp + half
        for c in (0, 4, 1, 7, 2, 6, 3, 5):
            er, ei = _dot(dc[c], mm(n1, 0)), _dot(dc[c], mm(n1, 1))
            br, bi = er[64:], ei[64:]
            if c == 0:
                fr[n1, 512:520, :] = br[:8]
                fi[n1, 512:520, :] = bi[:8]
                br = jnp.concatenate([jnp.where(row0, 0.0, br[:8]), br[8:]], axis=0)
                bi = jnp.concatenate([jnp.where(row0, 0.0, bi[:8]), bi[8:]], axis=0)
            fr[n1, c * 64:(c + 1) * 64, :] = er[:64] - bi
            fi[n1, c * 64:(c + 1) * 64, :] = ei[:64] + br


def _filter_block(r0, wr, wi, fr, fi):
    z = _fft16([(fr[n, pl.ds(r0, 8), :], fi[n, pl.ds(r0, 8), :]) for n in range(16)], -1)
    z = [(z[k][0] * wr[k] - z[k][1] * wi[k], z[k][0] * wi[k] + z[k][1] * wr[k]) for k in range(16)]
    z = _fft16(z, 1)
    for n in range(16):
        fr[n, pl.ds(r0, 8), :] = z[n][0]
        fi[n, pl.ds(r0, 8), :] = z[n][1]


def _filter_two_blocks(i, wra, wia, fr, fi, row0):
    rho, jb = i // 8, i % 8
    sc = jnp.where(jnp.logical_and(row0, i == 0), 0.5, 1.0)
    wr = [wra[k, pl.ds(rho + 32 * jb, 8, stride=4), :] for k in range(16)]
    wi = [wia[k, pl.ds(rho + 32 * jb, 8, stride=4), :] for k in range(16)]
    r0 = pl.multiple_of(rho * 128 + jb * 8, 8)
    _filter_block(r0, [_lo_f32(v) * sc for v in wr], [_lo_f32(v) * sc for v in wi], fr, fi)
    _filter_block(r0 + 64, [_hi_f32(v) for v in wr], [_hi_f32(v) for v in wi], fr, fi)


def _twiddle16(v, e, sgn):
    re, im = v
    if e == 0:
        return v
    if e == 4:
        return (im, -re) if sgn < 0 else (-im, re)
    if e == 2:
        return ((re + im) * RH, (im - re) * RH) if sgn < 0 else ((re - im) * RH, (im + re) * RH)
    if e == 6:
        return ((im - re) * RH, (re + im) * -RH) if sgn < 0 else ((re + im) * -RH, (re - im) * RH)
    c, s = float(np.cos(np.pi * e / 8)), float(sgn * np.sin(np.pi * e / 8))
    return (re * c - im * s, re * s + im * c)


def _filter_pieces(i, wra, wia, fr, fi, row0):
    rho, jb = i // 8, i % 8
    sc = jnp.where(jnp.logical_and(row0, i == 0), 0.5, 1.0)
    pieces = []
    for half, cvt in enumerate((_lo_f32, _hi_f32)):
        rows = pl.ds(pl.multiple_of(rho * 128 + jb * 8 + 64 * half, 8), 8)

        def load(ns, rows=rows):
            return [(fr[n, rows, :], fi[n, rows, :]) for n in ns]

        def store(ns, z, rows=rows):
            for n, (re, im) in zip(ns, z):
                fr[n, rows, :] = re
                fi[n, rows, :] = im

        def outer(a, sgn, load=load, store=store):
            ns = [a, a + 4, a + 8, a + 12]
            store(ns, _fft4(*load(ns), sgn))

        def inner(kl, half=half, cvt=cvt, load=load, store=store):
            ns = [4 * kl + a for a in range(4)]
            z = _fft4(*[_twiddle16(v, a * kl, -1) for a, v in enumerate(load(ns))], -1)
            y = []
            for kh in range(4):
                wr = cvt(wra[kl + 4 * kh, pl.ds(rho + 32 * jb, 8, stride=4), :])
                wi = cvt(wia[kl + 4 * kh, pl.ds(rho + 32 * jb, 8, stride=4), :])
                if half == 0:
                    wr, wi = wr * sc, wi * sc
                y.append((z[kh][0] * wr - z[kh][1] * wi, z[kh][0] * wi + z[kh][1] * wr))
            store(ns, [_twiddle16(v, a * kl, 1) for a, v in enumerate(_fft4(*y, 1))])

        pieces += [functools.partial(outer, a, -1) for a in range(4)]
        pieces += [functools.partial(inner, kl) for kl in range(4)]
        pieces += [functools.partial(outer, a, 1) for a in range(4)]
    return pieces


def _filter_nyquist(wr_ny, wi_ny, fr, fi):
    nr = wr_ny[...].astype(f32) * 0.5
    ni = wi_ny[...].astype(f32) * 0.5
    _filter_block(512, [nr[:, k * 128:(k + 1) * 128] for k in range(16)],
                  [ni[:, k * 128:(k + 1) * 128] for k in range(16)], fr, fi)


def _spectral_inverse(jp, fr, fi, g, mm, ya, row0):
    tcs = []
    for half in range(2):
        n1 = 2 * jp + half
        m2 = jnp.concatenate([mm(n1, 0), mm(n1, 1)], axis=1)
        tc = {}
        for c in (0, 4, 1, 7, 2, 6, 3, 5):
            br, bi = fr[n1, c * 64:(c + 1) * 64, :], fi[n1, c * 64:(c + 1) * 64, :]
            b1, b2 = bi, -br
            if c == 0:
                b1 = jnp.concatenate([jnp.where(row0, fr[n1, 512:520, :], b1[:8]), b1[8:]], axis=0)
                b2 = jnp.concatenate([jnp.where(row0, fi[n1, 512:520, :], b2[:8]), b2[8:]], axis=0)
            rhs = jnp.concatenate([jnp.concatenate([br, b1], axis=0),
                                   jnp.concatenate([bi, b2], axis=0)], axis=1).astype(bf16)
            tc[c] = _dot_t(m2, rhs)
        tcs.append(tc)
    vs = []
    for tc in tcs:
        v0, v4 = _dot(tc[0], g(0)), _dot(tc[4], g(1))
        pq = []
        for r in (1, 2, 3):
            o = 2 + 4 * (r - 1)
            pq.append((_dot(tc[r], g(o)) + _dot(tc[8 - r], g(o + 2)),
                       _dot(tc[r], g(o + 1)) + _dot(tc[8 - r], g(o + 3))))
        vs.append([v0, v4] + [t for both in pq for t in both])
    for r0 in range(0, 128, 8):
        ys = []
        for v in vs:
            v0, v4, p1, q1, p2, q2, p3, q3 = [t[r0:r0 + 8] for t in v]
            e0, e1 = v0 + v4, v0 - v4
            a0, a2, a1, a3 = e0 + p2, e0 - p2, e1 - q2, e1 + q2
            b0, b2 = p1 + p3, q3 - q1
            t0, t1 = p1 - p3, q1 + q3
            b1, b3 = (t0 - t1) * RH, (t0 + t1) * -RH
            ys.append([a0 + b0, a1 + b1, a2 + b2, a3 + b3, a0 - b0, a1 - b1, a2 - b2, a3 - b3])
        for t in range(8):
            lo = pltpu.bitcast(ys[0][t].astype(bf16).astype(f32), u32) >> 16
            hi = pltpu.bitcast(ys[1][t].astype(bf16).astype(f32), u32)
            ya[jp, pl.ds(r0, 8), pl.ds(t * 128, 128)] = lo | hi


def _repack_head_pair(w, j):
    for r0 in range(0, D, 16):
        even = w[j, pl.ds(r0, 8, stride=2), :]
        odd = w[j, pl.ds(r0 + 1, 8, stride=2), :]
        w[j, pl.ds(r0, 8), :] = (even & u32(0xFFFF)) | (odd << 16)
        w[j, pl.ds(r0 + 8, 8), :] = (even >> 16) | (odd & u32(0xFFFF0000))


def _head_weight(w, j, parity, k0=0, kn=D):
    return _every_other_tile(w[j, pl.ds(k0, kn), :], parity)


def _project_early_rows(j, xe, w, early):
    lhs = jnp.concatenate([pltpu.bitcast(xe[t], bf16) for t in range(8)], axis=1)
    for parity in range(2):
        early[2 * j + parity] = _dot(lhs, _head_weight(w, j, parity))


def _schedule():
    heads = lambda grp: range(grp * GH, (grp + 1) * GH)
    order = []
    if SCHED == 0:
        for t in range(NG + 3):
            if t < NG:
                order += [("P", h) for h in heads(t)]
            if 0 <= t - 1 < NG:
                order += [("S", h) for h in heads(t - 1)]
            if 0 <= t - 2 < NG:
                order += [("M", h) for h in heads(t - 2)]
            if 0 <= t - 3 < NG:
                order += [("O", t - 3, j) for j in range(8)]
            order.append(("X", t))
    elif SCHED == 1:
        for t in range(NG + 3):
            for i in range(GH):
                if t < NG:
                    order.append(("P", t * GH + i))
                if 0 <= t - 1 < NG:
                    order.append(("S", (t - 1) * GH + i))
                if 0 <= t - 2 < NG:
                    order.append(("M", (t - 2) * GH + i))
                if 0 <= t - 3 < NG:
                    order += [("O", t - 3, 2 * i), ("O", t - 3, 2 * i + 1)]
            order.append(("X", t))
    elif SCHED in (2, 3, 4):
        lag = SCHED + 2
        done = 0
        for t in range(NG):
            order += [("P", h) for h in heads(t)]
            if t >= 1:
                order += [("S", h) for h in heads(t - 1)]
            if t >= 2:
                order += [("M", h) for h in heads(t - 2)]
            if t >= lag:
                order += [("O", done, j) for j in range(8)]
                done += 1
            order.append(("X", t))
        order += [("O", done, j) for j in range(4)]
        order += [("S", h) for h in heads(NG - 1)] + [("M", h) for h in heads(NG - 2)]
        order += [("O", done, j) for j in range(4, 8)]
        done += 1
        while done < NG - 2:
            order += [("O", done, j) for j in range(8)]
            done += 1
        order += [("M", h) for h in heads(NG - 1)]
        order += [("O", grp, j) for grp in (NG - 2, NG - 1) for j in range(8)]
    elif SCHED == 5:
        for t in range(NG + 3):
            hs = list(heads(t)) if t < NG else []
            order += [("P", h) for h in hs[:2]]
            if 0 <= t - 1 < NG:
                order += [("S", h) for h in heads(t - 1)]
            if 0 <= t - 3 < NG:
                order += [("O", t - 3, j) for j in range(4)]
            order += [("P", h) for h in hs[2:]]
            if 0 <= t - 2 < NG:
                order += [("M", h) for h in heads(t - 2)]
            if 0 <= t - 3 < NG:
                order += [("O", t - 3, j) for j in range(4, 8)]
            order.append(("X", t))
    elif SCHED == 6:
        for t in range(NG + 2):
            if t < NG:
                order += [("P", h, "qk") for h in heads(t)]
            if 0 <= t - 1 < NG:
                order += [("M", h) for h in heads(t - 1)]
            if t < NG:
                order += [("P", h, "v") for h in list(heads(t))[:2]]
                order += [("S", h) for h in heads(t)]
                order += [("P", h, "v") for h in list(heads(t))[2:]]
            if 0 <= t - 1 < NG:
                order += [("O", t - 1, j) for j in range(8)]
            order.append(("X", t))
    return order


def _segment(s, mem, xl, w, wo, early, ob, mask, side_work):
    hh = jnp.concatenate([mem, xl[s].astype(f32)], axis=0).astype(LHS_DTYPE)
    e0 = pl.multiple_of(s * EARLY, EARLY)
    q, k, v, p, o = {}, {}, {}, {}, {}
    acc = [None] * 8
    heads = lambda grp: range(grp * GH, (grp + 1) * GH)

    first_half = {}
    for h in range(SPLIT_HEADS):
        for i in range(3):
            first_half[i, h] = _dot(hh[:, :D // 2], _head_weight(w, i * (H // 2) + h // 2, h % 2, 0, D // 2))

    def project_one(i, h):
        j = i * (H // 2) + h // 2
        if (i, h) in first_half:
            y = first_half[i, h] + _dot(hh[:, D // 2:], _head_weight(w, j, h % 2, D // 2, D // 2))
        else:
            y = _dot(hh, _head_weight(w, j, h % 2))
        return jnp.concatenate([y[:M], early[i * H + h, pl.ds(e0, EARLY), :], y[M:]], axis=0)

    def project(h, which="qkv"):
        if "q" in which:
            q[h] = project_one(0, h)
            if side_work.get("pieces") and h >= PACE_FROM:
                if FILTER_MODE == 2:
                    side_work["pace"](q[h][:8])
                side_work["pieces"].pop(0)()
        if "k" in which:
            k[h] = project_one(1, h).astype(bf16)
        if "v" in which:
            v[h] = project_one(2, h).astype(bf16)

    def softmax(h):
        if SOFTMAX == 0:
            sc = jnp.where(mask, _dot_t(q.pop(h), k.pop(h)) * DH ** -0.5, -1e9)
            e = jnp.exp(sc - jnp.max(sc, axis=1, keepdims=True))
            p[h] = e / jnp.sum(e, axis=1, keepdims=True)
        else:
            sc = jnp.where(mask, _dot_t(q.pop(h), k.pop(h)) * (DH ** -0.5 * LOG2E), -1e9 * LOG2E)
            e = jnp.exp2(sc - jnp.max(sc, axis=1, keepdims=True))
            total = jnp.sum(e, axis=1, keepdims=True)
            if SOFTMAX == 1:
                p[h] = e / total
            elif SOFTMAX == 2:
                r = pl.reciprocal(total, approx=True)
                p[h] = e * (r * (2.0 - total * r))
            else:
                r = pl.reciprocal(total, approx=True)
                p[h] = (e, r * (2.0 - total * r))

    def mix(h):
        if SOFTMAX == 3:
            e, r = p.pop(h)
            o[h] = _dot(e, v.pop(h)) * r
        else:
            o[h] = _dot(p.pop(h), v.pop(h))

    def out_project(grp, j):
        og = jnp.concatenate([o[h] for h in heads(grp)], axis=1)
        t = _dot(og, pltpu.bitcast(wo[j, pl.ds(grp * GH * DH // 2, GH * DH // 2), :], bf16))
        acc[j] = t if acc[j] is None else acc[j] + t

    ops = {"P": project, "S": softmax, "M": mix, "O": out_project, "X": lambda t: side_work.get(t, lambda: None)()}
    for op, *args in _schedule():
        ops[op](*args)
    res = jnp.concatenate(acc, axis=1)
    ob[pl.ds(2 * s, 2)] = res[M:].astype(bf16).reshape(2, 16, D)
    return res[:M].astype(bf16).astype(f32)


def _kernel(ax_hbm, wr_hbm, wi_hbm, g_hbm, mm_hbm,
            bx_hbm, m0_hbm, wq_hbm, wk_hbm, wv_hbm, wo_hbm, out_hbm,
            xa, wra, wia, wr_ny, wi_ny, g_ref, mm_ref, fr, fi, ya,
            w, wo, xe_raw, xe, xl, m0, early, ob, sems, ya_sem, ob_sem):
    n_pairs = 3 * H // 2
    n_sem = [n_pairs]

    def copy(src, dst):
        n_sem[0] += 1
        return pltpu.make_async_copy(src, dst, sems.at[n_sem[0] - 1])

    def lane_tile(t):
        return pl.ds(t * 128, 128)

    def start(copies):
        for c in copies:
            c.start()

    def wait(copies):
        for c in copies:
            c.wait()

    def wait_pair(j):
        pltpu.make_async_copy(w.at[j], w.at[j], sems.at[j]).wait()

    ax_words, out_words = ax_hbm.bitcast(u32), out_hbm.bitcast(u32)
    c_g = copy(g_hbm, g_ref)
    c_ax = [[copy(ax_words.at[:, jp, :], xa.at[jp]), copy(mm_hbm.at[pl.ds(4 * jp, 4)], mm_ref.at[pl.ds(4 * jp, 4)])]
            for jp in range(8)]
    c_xe = copy(bx_hbm.at[:, pl.ds(0, EARLY), :], xe_raw)
    c_w = [pltpu.make_async_copy(src.bitcast(u32).at[:, j, :], w.at[i * (H // 2) + j], sems.at[i * (H // 2) + j])
           for i, src in enumerate((wq_hbm, wk_hbm, wv_hbm)) for j in range(H // 2)]
    c_rest = [copy(wo_hbm.bitcast(u32).at[:, lane_tile(t)], wo.at[t]) for t in range(8)]
    c_rest += [copy(m0_hbm, m0), copy(bx_hbm.at[:, pl.ds(EARLY, SEG - EARLY), :], xl)]
    c_aw = [copy(src.at[pl.ds(0, 512), :].bitcast(u32).at[:, lane_tile(t)], dst.at[t])
            for src, dst in ((wr_hbm, wra), (wi_hbm, wia)) for t in range(16)]
    c_aw += [copy(wr_hbm.at[pl.ds(512, 1), :], wr_ny), copy(wi_hbm.at[pl.ds(512, 1), :], wi_ny)]
    start([c_g] + sum(c_ax, []) + [c_xe] + c_w[:24])

    row0 = lax.broadcasted_iota(jnp.int32, (8, 128), 0) == 0
    g = lambda i: pltpu.bitcast(g_ref[i], bf16)
    mm = lambda n1, part: pltpu.bitcast(mm_ref[2 * n1 + part], bf16)
    with jax.named_scope("p1_fwd"):
        wait([c_g] + c_ax[0])
        us = _forward_butterflies(0, xa)
        for group in FWD_GROUPS:
            wait(sum((c_ax[jp] for jp in group), []))
            for jp in group:
                _forward_matmuls(jp - 1, us, g, mm, fr, fi, row0)
                us = _forward_butterflies(jp, xa)
        start(c_w[24:] + c_rest)
        _forward_matmuls(7, us, g, mm, fr, fi, row0)

    with jax.named_scope("p2_xe"):
        c_xe.wait()
        wait_pair(0)
        for i in range(NSEG // 2):
            rows = jnp.concatenate([xe_raw[2 * i].astype(f32), xe_raw[2 * i + 1].astype(f32)], axis=0)
            words = pltpu.bitcast(rows.astype(bf16), u32)
            for t in range(8):
                xe[t, pl.ds(8 * i, 8), :] = words[:, t * 128:(t + 1) * 128]
        _repack_head_pair(w, 0)

    def project(i, _):
        for u in range(PAIRS_PER_ITER):
            wait_pair(i * PAIRS_PER_ITER + u + 1)
        for u in range(PAIRS_PER_ITER):
            j = i * PAIRS_PER_ITER + u
            _project_early_rows(j, xe, w, early)
            _repack_head_pair(w, j + 1)
        return 0

    n_iter = (n_pairs - 1) // PAIRS_PER_ITER
    with jax.named_scope("p3_proj"):
        lax.fori_loop(0, n_iter // 2, project, 0)
        start(c_aw)
        lax.fori_loop(n_iter // 2, n_iter, project, 0)
        for j in range(n_iter * PAIRS_PER_ITER + 1, n_pairs):
            wait_pair(j)
        for j in range(n_iter * PAIRS_PER_ITER, n_pairs):
            _project_early_rows(j, xe, w, early)
            if j + 1 < n_pairs:
                _repack_head_pair(w, j + 1)
    with jax.named_scope("p4_wait"):
        wait(c_rest + c_aw)
        _filter_nyquist(wr_ny, wi_ny, fr, fi)

    row = lax.broadcasted_iota(jnp.int32, (L, L), 0)
    col = lax.broadcasted_iota(jnp.int32, (L, L), 1)
    mask = (row < M) | (row >= col)

    def steps(with_filter, i, mem):
        for u in range(UNROLL):
            s = i * UNROLL + u
            side_work = {}
            if with_filter:
                if FILTER_MODE == 0:
                    side_work[FILTER_AT] = lambda s=s: _filter_two_blocks(s, wra, wia, fr, fi, row0)
                else:
                    side_work["pieces"] = _filter_pieces(s, wra, wia, fr, fi, row0)
                    side_work["pace"] = lambda val: (fr.__setitem__((0, slice(520, 528)), val), fi.__setitem__((0, slice(520, 528)), val))
            mem = _segment(s, mem, xl, w, wo, early, ob, mask, side_work)
        rows = pl.ds(2 * UNROLL * i, 2 * UNROLL)
        pltpu.make_async_copy(ob.at[rows], out_hbm.at[rows, :, pl.ds(D, D)], ob_sem).start()
        return mem

    with jax.named_scope("p5_steps"):
        mem = lax.fori_loop(0, 32 // UNROLL, functools.partial(steps, True), m0[...].astype(f32))
    c_ya = [pltpu.make_async_copy(ya.at[jp], out_words.at[:, jp, pl.ds(0, D)], ya_sem) for jp in range(8)]
    with jax.named_scope("p6_inv"):
        for jp in range(8):
            _spectral_inverse(jp, fr, fi, g, mm, ya, row0)
        start(c_ya)
    with jax.named_scope("p7_steps"):
        lax.fori_loop(32 // UNROLL, N_STEPS // UNROLL, functools.partial(steps, False), mem)
    wait(c_ya)
    pltpu.make_async_copy(ob.at[pl.ds(0, 2 * N_STEPS)], ob.at[pl.ds(0, 2 * N_STEPS)], ob_sem).wait()


def _run(A_x, A_w_r, A_w_i, B_x, B_mem0, B_Wq, B_Wk, B_Wv, B_Wo):
    hbm = pl.BlockSpec(memory_space=pltpu.HBM)
    out = pl.pallas_call(
        _kernel,
        out_shape=jax.ShapeDtypeStruct((S // 16, 16, 2 * D), bf16),
        in_specs=[hbm] * 11,
        out_specs=hbm,
        scratch_shapes=[
            pltpu.VMEM((8, 128, D), u32),
            pltpu.VMEM((16, 256, 128), u32),
            pltpu.VMEM((16, 256, 128), u32),
            pltpu.VMEM((1, S), bf16),
            pltpu.VMEM((1, S), bf16),
            pltpu.VMEM((14, 64, 128), u32),
            pltpu.VMEM((32, 64, 128), u32),
            pltpu.VMEM((16, 528, 128), f32),
            pltpu.VMEM((16, 528, 128), f32),
            pltpu.VMEM((8, 128, D), u32),
            pltpu.VMEM((3 * H // 2, D, 128), u32),
            pltpu.VMEM((8, H * DH // 2, 128), u32),
            pltpu.VMEM((NSEG, EARLY, D), bf16),
            pltpu.VMEM((8, NSEG * EARLY // 2, 128), u32),
            pltpu.VMEM((NSEG, SEG - EARLY, D), bf16),
            pltpu.VMEM((M, D), bf16),
            pltpu.VMEM((3 * H, NSEG * EARLY, DH), f32),
            pltpu.VMEM((S // 16, 16, D), bf16),
            pltpu.SemaphoreType.DMA((110,)),
            pltpu.SemaphoreType.DMA(()),
            pltpu.SemaphoreType.DMA(()),
        ],
        compiler_params=pltpu.CompilerParams(
            vmem_limit_bytes=120 * 1024 * 1024, flags=FLAGS),
        name="gfnet_rmt",
    )(A_x.reshape(S // 16, 16, D), A_w_r.T, A_w_i.T, _G_CONST, _MM_CONST,
      B_x.reshape(NSEG, SEG, D), B_mem0.reshape(M, D), B_Wq, B_Wk, B_Wv, B_Wo.reshape(H * DH, D))
    return out.reshape(1, S, 2 * D)


_run_jit = jax.jit(_run)


def pallas_concat_heads__spectral_gfnet__memory_aug_recurrent_mem_tr__prompt_kernel(
    A_x, A_w_r, A_w_i, B_x, B_mem0, B_Wq, B_Wk, B_Wv, B_Wo, B_seg_len,
):
    assert A_x.shape == (1, S, D) and B_x.shape == (1, S, D) and B_mem0.shape == (1, M, D)
    assert B_Wq.shape == (D, H, DH) and B_Wo.shape == (H, DH, D)
    assert B_seg_len == SEG, "the kernel is specialised to the problem's segment length"
    return _run_jit(A_x, A_w_r, A_w_i, B_x, B_mem0, B_Wq, B_Wk, B_Wv, B_Wo)
```

```python
import functools

import jax
import jax.numpy as jnp
import numpy as np
from jax import lax
import jax.experimental.pallas as pl
import jax.experimental.pallas.tpu as pltpu

f32, bf16, u32 = jnp.float32, jnp.bfloat16, jnp.uint32

S = 2048
D = 1024
H, DH = 32, 128
M = 8
SEG = 32
L = M + SEG
NSEG = S // SEG
EARLY = 8
GH = 4
NG = H // GH
UNROLL = 2
PAIRS = 6
N_PAIRS = 3 * H // 2

CLASS_PAIRS = ((0, 4), (1, 7), (2, 6), (3, 5))
NYQUIST_ROW = D // 2
PACE_ROW = NYQUIST_ROW + 8
RH = float(np.sqrt(0.5))
LOG2E = float(np.log2(np.e))
LO_MASK, HI_MASK = np.uint32(0xFFFF), np.uint32(0xFFFF0000)

FORWARD_PLAN = (
    ((0,), "b0 m0"),
    ((1,), "b1"),
    ((2,), "m1 b2"),
    ((3, 4), "m2 b3 m3 b4"),
    ((5, 6, 7), "m4 b5 m5 b6 m6 b7 m7"),
)


def _dot(a, b):
    return lax.dot_general(a, b, (((1,), (0,)), ((), ())), preferred_element_type=f32)


def _dot_t(a, b):
    return lax.dot_general(a, b, (((1,), (1,)), ((), ())), preferred_element_type=f32)


def _lo_f32(words):
    return pltpu.bitcast(words << 16, f32)


def _hi_f32(words):
    return pltpu.bitcast(words & HI_MASK, f32)


def _unit_roots(rows, n):
    shape = (rows, 128)
    turns = (lax.broadcasted_iota(jnp.int32, shape, 0) * lax.broadcasted_iota(jnp.int32, shape, 1)) & (n - 1)
    angle = turns.astype(f32) * (-2 * np.pi / n)
    return jnp.cos(angle), jnp.sin(angle)


def _put_bf16(ref, i, val):
    ref[i] = pltpu.bitcast(val.astype(bf16), u32)


def _rotate(re, im, twiddles, i):
    c, s = twiddles[0][i:i + 1], twiddles[1][i:i + 1]
    return re * c - im * s, re * s + im * c


def _make_d_matrices(g_ref, f_re, f_im):
    twiddles = _unit_roots(8, D)
    re, im = f_re[:72] * 2.0 ** -10, f_im[:64] * 2.0 ** -10
    cls = [_rotate(re[:64], im, twiddles, r) for r in range(8)]
    first = lax.broadcasted_iota(jnp.int32, (64, 128), 0) == 0
    _put_bf16(g_ref, 0, jnp.concatenate([cls[0][0], jnp.where(first, re[64:65], cls[0][1])], axis=0))
    _put_bf16(g_ref, 1, jnp.concatenate(cls[4], axis=0))
    for r in (1, 2, 3):
        (c, s), (c_, s_) = cls[r], cls[8 - r]
        _put_bf16(g_ref, 3 * r - 1, jnp.concatenate([c, c_], axis=0))
        _put_bf16(g_ref, 3 * r, jnp.concatenate([c + s, c_ - s_], axis=0))
        _put_bf16(g_ref, 3 * r + 1, jnp.concatenate([s - c, s_ + c_], axis=0))


def _make_s_matrices(mm_ref, n1, f_re, f_im, twiddles):
    parts = []
    for r0 in range(0, 128, 8):
        re, im = _rotate(f_re[r0:r0 + 8], f_im[r0:r0 + 8], twiddles, n1)
        parts.append((re, re + im, im - re, im))
    for i, tile in enumerate(zip(*parts)):
        _put_bf16(mm_ref, 4 * n1 + i, jnp.concatenate(tile, axis=0))


def _forward_butterflies(jp, xa):
    def rows(r0, cvt):
        x = [cvt(xa[jp, pl.ds(r0, 8), pl.ds(t * 128, 128)]) for t in range(8)]
        a = [x[i] + x[i + 4] for i in range(4)]
        b = [x[i] - x[i + 4] for i in range(4)]
        e0, e1 = a[0] + a[2], a[1] + a[3]
        t0, t1 = (b[1] - b[3]) * RH, (b[1] + b[3]) * -RH
        u = [e0 + e1, e0 - e1]
        for p, q in ((b[0] + t0, t1 - b[2]), (a[0] - a[2], a[3] - a[1]), (b[0] - t0, b[2] + t1)):
            u += [p + q, q, p]
        return u

    us = []
    for cvt in (_lo_f32, _hi_f32):
        parts = [rows(r0, cvt) for r0 in range(0, 128, 8)]
        us.append([jnp.concatenate(tile, axis=0).astype(bf16) for tile in zip(*parts)])
    return us


def _forward_matmuls(jp, us, g, mm, fr, fi, row0):
    spectra = []
    for u in us:
        d0, d4 = _dot_t(g(0), u[0]), _dot_t(g(1), u[1])
        nyquist = d0[64:72]
        x = [(jnp.concatenate([d0[:64], d4[:64]], axis=0),
              jnp.concatenate([jnp.where(row0, 0.0, nyquist), d0[72:], d4[64:]], axis=0))]
        for r in (1, 2, 3):
            t1, t2, t3 = [_dot_t(g(3 * r - 1 + i), u[3 * r - 1 + i]) for i in range(3)]
            x.append((t1 - t2, jnp.concatenate([t3[:64] + t1[:64], t3[64:] - t1[64:]], axis=0)))
        spectra.append((nyquist, x))
    for half, (nyquist, x) in enumerate(spectra):
        n1 = 2 * jp + half
        for classes, (re, im) in zip(CLASS_PAIRS, x):
            extra = [nyquist] if classes[0] == 0 else []
            t1 = _dot(jnp.concatenate([re + im] + extra, axis=0), mm(n1, 0))
            t2 = _dot(im, mm(n1, 1))
            t3 = _dot(jnp.concatenate([re] + extra, axis=0), mm(n1, 2))
            for i, c in enumerate(classes):
                rows = slice(64 * i, 64 * i + 64)
                fr[n1, pl.ds(64 * c, 64), :] = t1[rows] - t2[rows]
                fi[n1, pl.ds(64 * c, 64), :] = t1[rows] + t3[rows]
            if extra:
                fr[n1, pl.ds(NYQUIST_ROW, 8), :] = t1[128:]
                fi[n1, pl.ds(NYQUIST_ROW, 8), :] = t1[128:] + t3[128:]


def _fft4(z, sgn):
    a, b, c, d = z
    t0 = (a[0] + c[0], a[1] + c[1])
    t1 = (a[0] - c[0], a[1] - c[1])
    t2 = (b[0] + d[0], b[1] + d[1])
    t3 = (b[0] - d[0], b[1] - d[1])
    o0 = (t0[0] + t2[0], t0[1] + t2[1])
    o2 = (t0[0] - t2[0], t0[1] - t2[1])
    p = (t1[0] + t3[1], t1[1] - t3[0])
    m = (t1[0] - t3[1], t1[1] + t3[0])
    return (o0, p, o2, m) if sgn < 0 else (o0, m, o2, p)


def _twiddle16(v, e, sgn):
    re, im = v
    if e == 0:
        return v
    if e == 4:
        return (im, -re) if sgn < 0 else (-im, re)
    if e == 2:
        return ((re + im) * RH, (im - re) * RH) if sgn < 0 else ((re - im) * RH, (im + re) * RH)
    if e == 6:
        return ((im - re) * RH, (re + im) * -RH) if sgn < 0 else ((re + im) * -RH, (re - im) * RH)
    c, s = float(np.cos(np.pi * e / 8)), float(sgn * np.sin(np.pi * e / 8))
    return (re * c - im * s, re * s + im * c)


def _filter_pieces(r0, weight, fr, fi):
    rows = pl.ds(r0, 8)

    def load(ns):
        return [(fr[n, rows, :], fi[n, rows, :]) for n in ns]

    def store(ns, z):
        for n, (re, im) in zip(ns, z):
            fr[n, rows, :] = re
            fi[n, rows, :] = im

    def outer(a, sgn):
        ns = [a, a + 4, a + 8, a + 12]
        store(ns, _fft4(load(ns), sgn))

    def inner(kl):
        ns = [4 * kl + a for a in range(4)]
        z = _fft4([_twiddle16(v, a * kl, -1) for a, v in enumerate(load(ns))], -1)
        y = []
        for kh, (re, im) in enumerate(z):
            wr, wi = weight(kl + 4 * kh)
            y.append((re * wr - im * wi, re * wi + im * wr))
        store(ns, [_twiddle16(v, a * kl, 1) for a, v in enumerate(_fft4(y, 1))])

    return ([functools.partial(outer, a, -1) for a in range(4)]
            + [functools.partial(inner, kl) for kl in range(4)]
            + [functools.partial(outer, a, 1) for a in range(4)])


def _filter_two_classes(i, wra, wia, fr, fi, row0):
    rho, jb = i // 8, i % 8
    words = pl.ds(rho + 32 * jb, 8, stride=4)
    once = jnp.where(jnp.logical_and(row0, i == 0), 0.5, 1.0)
    even = lambda k: (_lo_f32(wra[k, words, :]) * once, _lo_f32(wia[k, words, :]) * once)
    odd = lambda k: (_hi_f32(wra[k, words, :]), _hi_f32(wia[k, words, :]))
    r0 = rho * 128 + jb * 8
    return (_filter_pieces(pl.multiple_of(r0, 8), even, fr, fi)
            + _filter_pieces(pl.multiple_of(r0 + 64, 8), odd, fr, fi))


def _filter_nyquist(wr_ny, wi_ny, fr, fi):
    wr, wi = wr_ny[...].astype(f32) * 0.5, wi_ny[...].astype(f32) * 0.5
    weight = lambda k: (wr[:, k * 128:(k + 1) * 128], wi[:, k * 128:(k + 1) * 128])
    for piece in _filter_pieces(NYQUIST_ROW, weight, fr, fi):
        piece()


def _inverse(jp, fr, fi, g, mm, ya, row0):
    sign = jnp.where(lax.broadcasted_iota(jnp.int32, (1, 128), 1) < 64, 1.0, -1.0)
    zs = []
    for n1 in (2 * jp, 2 * jp + 1):
        rows = lambda ref, c: ref[n1, pl.ds(64 * c, 64), :]
        z = {}
        for classes in CLASS_PAIRS[1:]:
            br = jnp.concatenate([rows(fr, c) for c in classes], axis=0)
            bi = jnp.concatenate([rows(fi, c) for c in classes], axis=0)
            t1 = _dot_t(mm(n1, 0), (br + bi).astype(bf16))
            z[classes[0]] = (t1 + _dot_t(mm(n1, 2), bi.astype(bf16)), t1 - _dot_t(mm(n1, 1), br.astype(bf16)))
        for c in (4, 0):
            br, bi = rows(fr, c), rows(fi, c)
            b1, b2 = bi, -br
            if c == 0:
                b1 = jnp.concatenate([jnp.where(row0, fr[n1, pl.ds(NYQUIST_ROW, 8), :], b1[:8]), b1[8:]], axis=0)
                b2 = jnp.concatenate([jnp.where(row0, fi[n1, pl.ds(NYQUIST_ROW, 8), :], b2[:8]), b2[8:]], axis=0)
            z[c] = (_dot_t(mm(n1, 0), jnp.concatenate([br, b1], axis=0).astype(bf16))
                    + _dot_t(mm(n1, 3), jnp.concatenate([bi, b2], axis=0).astype(bf16)))
        zs.append(z)
    vs = []
    for z in zs:
        v = []
        for r in (1, 2, 3):
            re, im = z[r]
            t1 = _dot(re + im * sign, g(3 * r - 1))
            v += [t1 + _dot(im, g(3 * r + 1)), t1 - _dot(re, g(3 * r))]
        vs.append(v + [_dot(z[4], g(1)), _dot(z[0], g(0))])
    for r0 in range(0, 128, 8):
        ys = []
        for v in vs:
            p1, q1, p2, q2, p3, q3, v4, v0 = [t[r0:r0 + 8] for t in v]
            e0, e1 = v0 + v4, v0 - v4
            a0, a2, a1, a3 = e0 + p2, e0 - p2, e1 - q2, e1 + q2
            b0, b2 = p1 + p3, q3 - q1
            t0, t1 = p1 - p3, q1 + q3
            b1, b3 = (t0 - t1) * RH, (t0 + t1) * -RH
            ys.append([a0 + b0, a1 + b1, a2 + b2, a3 + b3, a0 - b0, a1 - b1, a2 - b2, a3 - b3])
        for t in range(8):
            lo = pltpu.bitcast(ys[0][t].astype(bf16).astype(f32), u32) >> 16
            hi = pltpu.bitcast(ys[1][t].astype(bf16).astype(f32), u32)
            ya[jp, pl.ds(r0, 8), pl.ds(t * 128, 128)] = lo | hi


def _repack_head_pair(w, j):
    for r0 in range(0, D, 16):
        even = w[j, pl.ds(r0, 8, stride=2), :]
        odd = w[j, pl.ds(r0 + 1, 8, stride=2), :]
        w[j, pl.ds(r0, 8), :] = (even & LO_MASK) | (odd << 16)
        w[j, pl.ds(r0 + 8, 8), :] = (even >> 16) | (odd & HI_MASK)


def _head_weight(w, j, parity):
    words = w[j].reshape(D // 16, 2, 8, DH)[:, parity].reshape(D // 2, DH)
    return pltpu.bitcast(words, bf16)


def _project_early_rows(j, xe, w, early):
    lhs = jnp.concatenate([pltpu.bitcast(xe[t], bf16) for t in range(8)], axis=1)
    for parity in range(2):
        early[2 * j + parity] = _dot(lhs, _head_weight(w, j, parity))


def _segment(s, mem, xl, w, wo, early, ob, mask, side_work):
    hh = jnp.concatenate([mem, xl[s].astype(f32)], axis=0).astype(bf16)
    early_rows = pl.ds(pl.multiple_of(s * EARLY, EARLY), EARLY)
    q, k, v, p, o = {}, {}, {}, {}, {}
    acc = [None] * 8
    heads = lambda grp: range(grp * GH, (grp + 1) * GH)

    def project_one(i, h):
        y = _dot(hh, _head_weight(w, i * (H // 2) + h // 2, h % 2))
        return jnp.concatenate([y[:M], early[i * H + h, early_rows, :], y[M:]], axis=0)

    def project(grp):
        for h in heads(grp):
            q[h] = project_one(0, h)
            k[h] = project_one(1, h).astype(bf16)
            v[h] = project_one(2, h).astype(bf16)

    def softmax(grp):
        for h in heads(grp):
            scores = jnp.where(mask, _dot_t(q.pop(h), k.pop(h)) * (DH ** -0.5 * LOG2E), -1e9 * LOG2E)
            e = jnp.exp2(scores - jnp.max(scores, axis=1, keepdims=True))
            total = jnp.sum(e, axis=1, keepdims=True)
            r = pl.reciprocal(total, approx=True)
            p[h] = e * (r * (2.0 - total * r))

    def mix(grp):
        for h in heads(grp):
            o[h] = _dot(p.pop(h), v.pop(h))

    def out_project(grp, tiles=range(8)):
        og = jnp.concatenate([o[h] for h in heads(grp)], axis=1)
        for j in tiles:
            t = _dot(og, pltpu.bitcast(wo[j, pl.ds(grp * GH * DH // 2, GH * DH // 2), :], bf16))
            acc[j] = t if acc[j] is None else acc[j] + t
            if j < 4:
                side_work(t[:8])

    for t in range(NG):
        project(t)
        if t >= 1:
            softmax(t - 1)
        if t >= 2:
            mix(t - 2)
        if t >= 4:
            out_project(t - 4)
    out_project(NG - 4, range(4))
    softmax(NG - 1)
    mix(NG - 2)
    out_project(NG - 4, range(4, 8))
    out_project(NG - 3)
    mix(NG - 1)
    out_project(NG - 2)
    out_project(NG - 1)

    res = jnp.concatenate(acc, axis=1)
    ob[pl.ds(2 * s, 2)] = res[M:].astype(bf16).reshape(2, SEG // 2, D)
    return res[:M].astype(bf16).astype(f32)


def _kernel(ax_hbm, wr_hbm, wi_hbm, bx_hbm, m0_hbm, wq_hbm, wk_hbm, wv_hbm, wo_hbm, out_hbm,
            xa, wra, wia, wr_ny, wi_ny, g_ref, mm_ref, fr, fi, ya,
            w, wo, xe_raw, xe, xl, m0, early, ob, sems, ya_sem, ob_sem):
    sem_xe, sem_rest, sem_w = 8, 9, 10

    def copy(src, dst, sem):
        return pltpu.make_async_copy(src, dst, sems.at[sem])

    def lane_tile(t):
        return pl.ds(t * 128, 128)

    def start(copies):
        for c in copies:
            c.start()

    def wait(copies):
        for c in copies:
            c.wait()

    c_ax = [copy(ax_hbm.bitcast(u32).at[:, jp, :], xa.at[jp], jp) for jp in range(8)]
    c_xe = copy(bx_hbm.at[:, pl.ds(0, EARLY), :], xe_raw, sem_xe)
    c_w = [copy(src.bitcast(u32).at[:, j, :], w.at[i * (H // 2) + j], sem_w + (i * (H // 2) + j) // PAIRS)
           for i, src in enumerate((wq_hbm, wk_hbm, wv_hbm)) for j in range(H // 2)]
    c_rest = [copy(wo_hbm.bitcast(u32).at[:, lane_tile(t)], wo.at[t], sem_rest) for t in range(8)]
    c_rest += [copy(m0_hbm, m0, sem_rest), copy(bx_hbm.at[:, pl.ds(EARLY, SEG - EARLY), :], xl, sem_rest)]
    c_aw = [copy(src.at[pl.ds(0, D // 2), :].bitcast(u32).at[:, lane_tile(t)], dst.at[t], sem_rest)
            for src, dst in ((wr_hbm, wra), (wi_hbm, wia)) for t in range(16)]
    c_aw += [copy(wr_hbm.at[pl.ds(D // 2, 1), :], wr_ny, sem_rest),
             copy(wi_hbm.at[pl.ds(D // 2, 1), :], wi_ny, sem_rest)]
    start(c_ax + [c_xe] + c_w[:N_PAIRS // 2])

    row0 = lax.broadcasted_iota(jnp.int32, (8, 128), 0) == 0
    g = lambda i: pltpu.bitcast(g_ref[i], bf16)
    mm = lambda n1, part: pltpu.bitcast(mm_ref[4 * n1 + part], bf16)
    f_re, f_im = _unit_roots(128, 128)
    s_twiddles = _unit_roots(16, S)
    _make_d_matrices(g_ref, f_re, f_im)
    for n1 in range(4):
        _make_s_matrices(mm_ref, n1, f_re, f_im, s_twiddles)
    us = {}
    for arrived, stages in FORWARD_PLAN:
        wait([c_ax[jp] for jp in arrived])
        if 7 in arrived:
            c_xe.wait()
            start(c_w[N_PAIRS // 2:] + c_rest)
        for stage in stages.split():
            jp = int(stage[1])
            if stage[0] == "m":
                _forward_matmuls(jp, us.pop(jp), g, mm, fr, fi, row0)
                continue
            us[jp] = _forward_butterflies(jp, xa)
            for n1 in range(max(2 * jp, 4), 2 * jp + 2):
                _make_s_matrices(mm_ref, n1, f_re, f_im, s_twiddles)

    for i in range(NSEG // 2):
        rows = jnp.concatenate([xe_raw[2 * i].astype(f32), xe_raw[2 * i + 1].astype(f32)], axis=0)
        words = pltpu.bitcast(rows.astype(bf16), u32)
        for t in range(8):
            xe[t, pl.ds(8 * i, 8), :] = words[:, t * 128:(t + 1) * 128]

    def project_early(i, _):
        group = w.at[pl.ds(i * PAIRS, PAIRS)]
        pltpu.make_async_copy(group, group, sems.at[sem_w + i]).wait()

        @pl.when(i == N_PAIRS // PAIRS // 2)
        def _():
            start(c_aw)

        for u in range(PAIRS):
            _repack_head_pair(w, i * PAIRS + u)
            _project_early_rows(i * PAIRS + u, xe, w, early)
        return 0

    lax.fori_loop(0, N_PAIRS // PAIRS, project_early, 0)
    wait(c_rest + c_aw)

    row = lax.broadcasted_iota(jnp.int32, (L, L), 0)
    col = lax.broadcasted_iota(jnp.int32, (L, L), 1)
    mask = (row < M) | (row >= col)

    def segments(with_filter, i, mem):
        for s in [i * UNROLL + u for u in range(UNROLL)]:
            pieces = _filter_two_classes(s, wra, wia, fr, fi, row0) if with_filter else []

            def side_work(fresh):
                if pieces:
                    fr[0, pl.ds(PACE_ROW, 8), :] = fresh
                    fi[0, pl.ds(PACE_ROW, 8), :] = fresh
                    pieces.pop(0)()

            mem = _segment(s, mem, xl, w, wo, early, ob, mask, side_work)
            assert not pieces
        rows = pl.ds(2 * UNROLL * i, 2 * UNROLL)
        pltpu.make_async_copy(ob.at[rows], out_hbm.at[rows, :, pl.ds(D, D)], ob_sem).start()
        return mem

    mem = lax.fori_loop(0, 32 // UNROLL, functools.partial(segments, True), m0[...].astype(f32))

    _filter_nyquist(wr_ny, wi_ny, fr, fi)
    for jp in range(8):
        _inverse(jp, fr, fi, g, mm, ya, row0)
    c_ya = [pltpu.make_async_copy(ya.at[jp], out_hbm.bitcast(u32).at[:, jp, pl.ds(0, D)], ya_sem)
            for jp in range(8)]
    start(c_ya)

    lax.fori_loop(32 // UNROLL, NSEG // UNROLL, functools.partial(segments, False), mem)
    wait(c_ya)
    pltpu.make_async_copy(ob, ob, ob_sem).wait()


def _run(A_x, A_w_r, A_w_i, B_x, B_mem0, B_Wq, B_Wk, B_Wv, B_Wo):
    hbm = pl.BlockSpec(memory_space=pltpu.HBM)
    out = pl.pallas_call(
        _kernel,
        out_shape=jax.ShapeDtypeStruct((S // 16, 16, 2 * D), bf16),
        in_specs=[hbm] * 9,
        out_specs=hbm,
        scratch_shapes=[
            pltpu.VMEM((8, 128, D), u32),
            pltpu.VMEM((16, D // 4, 128), u32),
            pltpu.VMEM((16, D // 4, 128), u32),
            pltpu.VMEM((1, S), bf16),
            pltpu.VMEM((1, S), bf16),
            pltpu.VMEM((11, 64, 128), u32),
            pltpu.VMEM((64, 64, 128), u32),
            pltpu.VMEM((16, PACE_ROW + 8, 128), f32),
            pltpu.VMEM((16, PACE_ROW + 8, 128), f32),
            pltpu.VMEM((8, 128, D), u32),
            pltpu.VMEM((N_PAIRS, D, DH), u32),
            pltpu.VMEM((8, H * DH // 2, 128), u32),
            pltpu.VMEM((NSEG, EARLY, D), bf16),
            pltpu.VMEM((8, NSEG * EARLY // 2, 128), u32),
            pltpu.VMEM((NSEG, SEG - EARLY, D), bf16),
            pltpu.VMEM((M, D), bf16),
            pltpu.VMEM((3 * H, NSEG * EARLY, DH), f32),
            pltpu.VMEM((S // 16, 16, D), bf16),
            pltpu.SemaphoreType.DMA((10 + N_PAIRS // PAIRS,)),
            pltpu.SemaphoreType.DMA(()),
            pltpu.SemaphoreType.DMA(()),
        ],
        compiler_params=pltpu.CompilerParams(vmem_limit_bytes=120 * 1024 * 1024),
        name="gfnet_rmt",
    )(A_x.reshape(S // 16, 16, D), A_w_r.T, A_w_i.T, B_x.reshape(NSEG, SEG, D), B_mem0.reshape(M, D),
      B_Wq, B_Wk, B_Wv, B_Wo.reshape(H * DH, D))
    return out.reshape(1, S, 2 * D)


_run_jit = jax.jit(_run)


def pallas_concat_heads__spectral_gfnet__memory_aug_recurrent_mem_tr__prompt_kernel(
    A_x, A_w_r, A_w_i, B_x, B_mem0, B_Wq, B_Wk, B_Wv, B_Wo, B_seg_len,
):
    assert A_x.shape == (1, S, D) and B_x.shape == (1, S, D) and B_mem0.shape == (1, M, D)
    assert B_Wq.shape == (D, H, DH) and B_Wo.shape == (H, DH, D)
    assert B_seg_len == SEG, "the kernel is built for the problem's segment length"
    return _run_jit(A_x, A_w_r, A_w_i, B_x, B_mem0, B_Wq, B_Wk, B_Wv, B_Wo)
```

```python
import functools

import jax
import jax.numpy as jnp
import numpy as np
from jax import lax
import jax.experimental.pallas as pl
import jax.experimental.pallas.tpu as pltpu

f32, bf16, u32 = jnp.float32, jnp.bfloat16, jnp.uint32

S = 2048
D = 1024
H, DH = 32, 128
M = 8
SEG = 32
L = M + SEG
NSEG = S // SEG
EARLY = 8
GH = 4
NG = H // GH
UNROLL = 2
PAIRS = 6
N_PAIRS = 3 * H // 2

CLASS_PAIRS = ((0, 4), (1, 7), (2, 6), (3, 5))
NYQUIST_ROW = D // 2
PACE_ROW = NYQUIST_ROW + 8
RH = float(np.sqrt(0.5))
LOG2E = float(np.log2(np.e))
LO_MASK, HI_MASK = np.uint32(0xFFFF), np.uint32(0xFFFF0000)

FORWARD_PLAN = (
    ((0,), "b0 m0"),
    ((1,), "b1"),
    ((2,), "m1 b2"),
    ((3, 4), "m2 b3 m3 b4"),
    ((5, 6, 7), "m4 b5 m5 b6 m6 b7 m7"),
)


def _dot(a, b):
    return lax.dot_general(a, b, (((1,), (0,)), ((), ())), preferred_element_type=f32)


def _dot_t(a, b):
    return lax.dot_general(a, b, (((1,), (1,)), ((), ())), preferred_element_type=f32)


def _lo_f32(words):
    return pltpu.bitcast(words << 16, f32)


def _hi_f32(words):
    return pltpu.bitcast(words & HI_MASK, f32)


def _unit_roots(rows, n):
    shape = (rows, 128)
    turns = (lax.broadcasted_iota(jnp.int32, shape, 0) * lax.broadcasted_iota(jnp.int32, shape, 1)) & (n - 1)
    angle = turns.astype(f32) * (-2 * np.pi / n)
    return jnp.cos(angle), jnp.sin(angle)


def _put_bf16(ref, i, val):
    ref[i] = pltpu.bitcast(val.astype(bf16), u32)


def _rotate(re, im, twiddles, i):
    c, s = twiddles[0][i:i + 1], twiddles[1][i:i + 1]
    return re * c - im * s, re * s + im * c


def _make_d_matrices(g_ref, f_re, f_im):
    twiddles = _unit_roots(8, D)
    re, im = f_re[:72] * 2.0 ** -10, f_im[:64] * 2.0 ** -10
    cls = [_rotate(re[:64], im, twiddles, r) for r in range(8)]
    first = lax.broadcasted_iota(jnp.int32, (64, 128), 0) == 0
    _put_bf16(g_ref, 0, jnp.concatenate([cls[0][0], jnp.where(first, re[64:65], cls[0][1])], axis=0))
    _put_bf16(g_ref, 1, jnp.concatenate(cls[4], axis=0))
    for r in (1, 2, 3):
        (c, s), (c_, s_) = cls[r], cls[8 - r]
        _put_bf16(g_ref, 3 * r - 1, jnp.concatenate([c, c_], axis=0))
        _put_bf16(g_ref, 3 * r, jnp.concatenate([c + s, c_ - s_], axis=0))
        _put_bf16(g_ref, 3 * r + 1, jnp.concatenate([s - c, s_ + c_], axis=0))


def _make_s_matrices(mm_ref, n1, f_re, f_im, twiddles):
    parts = []
    for r0 in range(0, 128, 8):
        re, im = _rotate(f_re[r0:r0 + 8], f_im[r0:r0 + 8], twiddles, n1)
        parts.append((re, re + im, im - re, im))
    for i, tile in enumerate(zip(*parts)):
        _put_bf16(mm_ref, 4 * n1 + i, jnp.concatenate(tile, axis=0))


def _forward_butterflies(jp, xa):
    def rows(r0, cvt):
        x = [cvt(xa[jp, pl.ds(r0, 8), pl.ds(t * 128, 128)]) for t in range(8)]
        a = [x[i] + x[i + 4] for i in range(4)]
        b = [x[i] - x[i + 4] for i in range(4)]
        e0, e1 = a[0] + a[2], a[1] + a[3]
        t0, t1 = (b[1] - b[3]) * RH, (b[1] + b[3]) * -RH
        u = [e0 + e1, e0 - e1]
        for p, q in ((b[0] + t0, t1 - b[2]), (a[0] - a[2], a[3] - a[1]), (b[0] - t0, b[2] + t1)):
            u += [p + q, q, p]
        return u

    us = []
    for cvt in (_lo_f32, _hi_f32):
        parts = [rows(r0, cvt) for r0 in range(0, 128, 8)]
        us.append([jnp.concatenate(tile, axis=0).astype(bf16) for tile in zip(*parts)])
    return us


def _forward_matmuls(jp, us, g, mm, fr, fi, row0):
    spectra = []
    for u in us:
        d0, d4 = _dot_t(g(0), u[0]), _dot_t(g(1), u[1])
        nyquist = d0[64:72]
        x = [(jnp.concatenate([d0[:64], d4[:64]], axis=0),
              jnp.concatenate([jnp.where(row0, 0.0, nyquist), d0[72:], d4[64:]], axis=0))]
        for r in (1, 2, 3):
            t1, t2, t3 = [_dot_t(g(3 * r - 1 + i), u[3 * r - 1 + i]) for i in range(3)]
            x.append((t1 - t2, jnp.concatenate([t3[:64] + t1[:64], t3[64:] - t1[64:]], axis=0)))
        spectra.append((nyquist, x))
    for half, (nyquist, x) in enumerate(spectra):
        n1 = 2 * jp + half
        for classes, (re, im) in zip(CLASS_PAIRS, x):
            extra = [nyquist] if classes[0] == 0 else []
            t1 = _dot(jnp.concatenate([re + im] + extra, axis=0), mm(n1, 0))
            t2 = _dot(im, mm(n1, 1))
            t3 = _dot(jnp.concatenate([re] + extra, axis=0), mm(n1, 2))
            for i, c in enumerate(classes):
                rows = slice(64 * i, 64 * i + 64)
                fr[n1, pl.ds(64 * c, 64), :] = t1[rows] - t2[rows]
                fi[n1, pl.ds(64 * c, 64), :] = t1[rows] + t3[rows]
            if extra:
                fr[n1, pl.ds(NYQUIST_ROW, 8), :] = t1[128:]
                fi[n1, pl.ds(NYQUIST_ROW, 8), :] = t1[128:] + t3[128:]


def _fft4(z, sgn):
    a, b, c, d = z
    t0 = (a[0] + c[0], a[1] + c[1])
    t1 = (a[0] - c[0], a[1] - c[1])
    t2 = (b[0] + d[0], b[1] + d[1])
    t3 = (b[0] - d[0], b[1] - d[1])
    o0 = (t0[0] + t2[0], t0[1] + t2[1])
    o2 = (t0[0] - t2[0], t0[1] - t2[1])
    p = (t1[0] + t3[1], t1[1] - t3[0])
    m = (t1[0] - t3[1], t1[1] + t3[0])
    return (o0, p, o2, m) if sgn < 0 else (o0, m, o2, p)


def _twiddle16(v, e, sgn):
    re, im = v
    if e == 0:
        return v
    if e == 4:
        return (im, -re) if sgn < 0 else (-im, re)
    if e == 2:
        return ((re + im) * RH, (im - re) * RH) if sgn < 0 else ((re - im) * RH, (im + re) * RH)
    if e == 6:
        return ((im - re) * RH, (re + im) * -RH) if sgn < 0 else ((re + im) * -RH, (re - im) * RH)
    c, s = float(np.cos(np.pi * e / 8)), float(sgn * np.sin(np.pi * e / 8))
    return (re * c - im * s, re * s + im * c)


def _filter_pieces(r0, weight, fr, fi):
    rows = pl.ds(r0, 8)

    def load(ns):
        return [(fr[n, rows, :], fi[n, rows, :]) for n in ns]

    def store(ns, z):
        for n, (re, im) in zip(ns, z):
            fr[n, rows, :] = re
            fi[n, rows, :] = im

    def outer(a, sgn):
        ns = [a, a + 4, a + 8, a + 12]
        store(ns, _fft4(load(ns), sgn))

    def inner(kl):
        ns = [4 * kl + a for a in range(4)]
        z = _fft4([_twiddle16(v, a * kl, -1) for a, v in enumerate(load(ns))], -1)
        y = []
        for kh, (re, im) in enumerate(z):
            wr, wi = weight(kl + 4 * kh)
            y.append((re * wr - im * wi, re * wi + im * wr))
        store(ns, [_twiddle16(v, a * kl, 1) for a, v in enumerate(_fft4(y, 1))])

    return ([functools.partial(outer, a, -1) for a in range(4)]
            + [functools.partial(inner, kl) for kl in range(4)]
            + [functools.partial(outer, a, 1) for a in range(4)])


def _filter_two_classes(i, wra, wia, fr, fi, row0):
    rho, jb = i // 8, i % 8
    words = pl.ds(rho + 32 * jb, 8, stride=4)
    once = jnp.where(jnp.logical_and(row0, i == 0), 0.5, 1.0)
    even = lambda k: (_lo_f32(wra[k, words, :]) * once, _lo_f32(wia[k, words, :]) * once)
    odd = lambda k: (_hi_f32(wra[k, words, :]), _hi_f32(wia[k, words, :]))
    r0 = rho * 128 + jb * 8
    return (_filter_pieces(pl.multiple_of(r0, 8), even, fr, fi)
            + _filter_pieces(pl.multiple_of(r0 + 64, 8), odd, fr, fi))


def _filter_nyquist(wr_ny, wi_ny, fr, fi):
    wr, wi = wr_ny[...].astype(f32) * 0.5, wi_ny[...].astype(f32) * 0.5
    weight = lambda k: (wr[:, k * 128:(k + 1) * 128], wi[:, k * 128:(k + 1) * 128])
    for piece in _filter_pieces(NYQUIST_ROW, weight, fr, fi):
        piece()


def _inverse(jp, fr, fi, g, mm, ya, row0):
    sign = jnp.where(lax.broadcasted_iota(jnp.int32, (1, 128), 1) < 64, 1.0, -1.0)
    zs = []
    for n1 in (2 * jp, 2 * jp + 1):
        rows = lambda ref, c: ref[n1, pl.ds(64 * c, 64), :]
        z = {}
        for classes in CLASS_PAIRS[1:]:
            br = jnp.concatenate([rows(fr, c) for c in classes], axis=0)
            bi = jnp.concatenate([rows(fi, c) for c in classes], axis=0)
            t1 = _dot_t(mm(n1, 0), (br + bi).astype(bf16))
            z[classes[0]] = (t1 + _dot_t(mm(n1, 2), bi.astype(bf16)), t1 - _dot_t(mm(n1, 1), br.astype(bf16)))
        for c in (4, 0):
            br, bi = rows(fr, c), rows(fi, c)
            b1, b2 = bi, -br
            if c == 0:
                b1 = jnp.concatenate([jnp.where(row0, fr[n1, pl.ds(NYQUIST_ROW, 8), :], b1[:8]), b1[8:]], axis=0)
                b2 = jnp.concatenate([jnp.where(row0, fi[n1, pl.ds(NYQUIST_ROW, 8), :], b2[:8]), b2[8:]], axis=0)
            z[c] = (_dot_t(mm(n1, 0), jnp.concatenate([br, b1], axis=0).astype(bf16))
                    + _dot_t(mm(n1, 3), jnp.concatenate([bi, b2], axis=0).astype(bf16)))
        zs.append(z)
    vs = []
    for z in zs:
        v = []
        for r in (1, 2, 3):
            re, im = z[r]
            t1 = _dot(re + im * sign, g(3 * r - 1))
            v += [t1 + _dot(im, g(3 * r + 1)), t1 - _dot(re, g(3 * r))]
        vs.append(v + [_dot(z[4], g(1)), _dot(z[0], g(0))])
    for r0 in range(0, 128, 8):
        ys = []
        for v in vs:
            p1, q1, p2, q2, p3, q3, v4, v0 = [t[r0:r0 + 8] for t in v]
            e0, e1 = v0 + v4, v0 - v4
            a0, a2, a1, a3 = e0 + p2, e0 - p2, e1 - q2, e1 + q2
            b0, b2 = p1 + p3, q3 - q1
            t0, t1 = p1 - p3, q1 + q3
            b1, b3 = (t0 - t1) * RH, (t0 + t1) * -RH
            ys.append([a0 + b0, a1 + b1, a2 + b2, a3 + b3, a0 - b0, a1 - b1, a2 - b2, a3 - b3])
        for t in range(8):
            lo = pltpu.bitcast(ys[0][t].astype(bf16).astype(f32), u32) >> 16
            hi = pltpu.bitcast(ys[1][t].astype(bf16).astype(f32), u32)
            ya[jp, pl.ds(r0, 8), pl.ds(t * 128, 128)] = lo | hi


def _repack_head_pair(w, j):
    for r0 in range(0, D, 16):
        even = w[j, pl.ds(r0, 8, stride=2), :]
        odd = w[j, pl.ds(r0 + 1, 8, stride=2), :]
        w[j, pl.ds(r0, 8), :] = (even & LO_MASK) | (odd << 16)
        w[j, pl.ds(r0 + 8, 8), :] = (even >> 16) | (odd & HI_MASK)


def _head_weight(w, j, parity):
    words = w[j].reshape(D // 16, 2, 8, DH)[:, parity].reshape(D // 2, DH)
    return pltpu.bitcast(words, bf16)


def _make_early_operands(xe_raw, xe):
    for i in range(NSEG // 4):
        top, bottom = [jnp.concatenate([xe_raw[s].astype(f32), xe_raw[s + 1].astype(f32)], axis=0)
                       for s in (2 * i, NSEG // 2 + 2 * i)]
        for t in range(4):
            a11, a12, a21, a22 = [half[:, c:c + 128] for half in (top, bottom)
                                  for c in (t * 128, D // 2 + t * 128)]
            for n, val in enumerate((a11 + a22, a21 + a22, a11, a22, a11 + a12, a21 - a11, a12 - a22)):
                xe[n, t, pl.ds(8 * i, 8), :] = pltpu.bitcast(val.astype(bf16), u32)


def _project_early_rows(j, xe, w, early):
    b11, b12 = (lambda r0, cvt=cvt: cvt(w[j, pl.ds(r0, 8), :]) for cvt in (_lo_f32, _hi_f32))
    b21, b22 = (lambda r0, cvt=cvt: cvt(w[j, pl.ds(D // 2 + r0, 8), :]) for cvt in (_lo_f32, _hi_f32))

    def product(n, right):
        total = None
        for t in range(4):
            tile = jnp.concatenate([right(r0) for r0 in range(t * 128, t * 128 + 128, 8)], axis=0)
            part = _dot(pltpu.bitcast(xe[n, t], bf16), tile.astype(bf16))
            total = part if total is None else total + part
        return total

    half = NSEG * EARLY // 2
    m1 = product(0, lambda r: b11(r) + b22(r))
    m4 = product(3, lambda r: b21(r) - b11(r))
    c11 = m1 + m4 + product(6, lambda r: b21(r) + b22(r))
    m5 = product(4, b22)
    early[2 * j, pl.ds(0, half), :] = c11 - m5
    m3 = product(2, lambda r: b12(r) - b22(r))
    early[2 * j + 1, pl.ds(0, half), :] = m3 + m5
    m2 = product(1, b11)
    early[2 * j, pl.ds(half, half), :] = m2 + m4
    early[2 * j + 1, pl.ds(half, half), :] = m1 + m3 - m2 + product(5, lambda r: b11(r) + b12(r))


def _segment(s, mem, xl, w, wo, early, ob, mask, side_work):
    hh = jnp.concatenate([mem, xl[s].astype(f32)], axis=0).astype(bf16)
    early_rows = pl.ds(pl.multiple_of(s * EARLY, EARLY), EARLY)
    q, k, v, p, o = {}, {}, {}, {}, {}
    acc = [None] * 8
    heads = lambda grp: range(grp * GH, (grp + 1) * GH)

    def project_one(i, h):
        y = _dot(hh, _head_weight(w, i * (H // 2) + h // 2, h % 2))
        return jnp.concatenate([y[:M], early[i * H + h, early_rows, :], y[M:]], axis=0)

    def project(grp):
        for h in heads(grp):
            q[h] = project_one(0, h)
            k[h] = project_one(1, h).astype(bf16)
            v[h] = project_one(2, h).astype(bf16)

    def softmax(grp):
        for h in heads(grp):
            scores = jnp.where(mask, _dot_t(q.pop(h), k.pop(h)) * (DH ** -0.5 * LOG2E), -1e9 * LOG2E)
            e = jnp.exp2(scores - jnp.max(scores, axis=1, keepdims=True))
            total = jnp.sum(e, axis=1, keepdims=True)
            r = pl.reciprocal(total, approx=True)
            p[h] = e * (r * (2.0 - total * r))

    def mix(grp):
        for h in heads(grp):
            o[h] = _dot(p.pop(h), v.pop(h))

    def out_project(grp, tiles=range(8)):
        og = jnp.concatenate([o[h] for h in heads(grp)], axis=1)
        for j in tiles:
            t = _dot(og, pltpu.bitcast(wo[j, pl.ds(grp * GH * DH // 2, GH * DH // 2), :], bf16))
            acc[j] = t if acc[j] is None else acc[j] + t
            if j < 4:
                side_work(t[:8])

    for t in range(NG):
        project(t)
        if t >= 1:
            softmax(t - 1)
        if t >= 2:
            mix(t - 2)
        if t >= 4:
            out_project(t - 4)
    out_project(NG - 4, range(4))
    softmax(NG - 1)
    mix(NG - 2)
    out_project(NG - 4, range(4, 8))
    out_project(NG - 3)
    mix(NG - 1)
    out_project(NG - 2)
    out_project(NG - 1)

    res = jnp.concatenate(acc, axis=1)
    ob[pl.ds(2 * s, 2)] = res[M:].astype(bf16).reshape(2, SEG // 2, D)
    return res[:M].astype(bf16).astype(f32)


def _kernel(ax_hbm, wr_hbm, wi_hbm, bx_hbm, m0_hbm, wq_hbm, wk_hbm, wv_hbm, wo_hbm, out_hbm,
            xa, wra, wia, wr_ny, wi_ny, g_ref, mm_ref, fr, fi, ya,
            w, wo, xe_raw, xe, xl, m0, early, ob, sems, ya_sem, ob_sem):
    sem_xe, sem_rest, sem_w = 8, 9, 10

    def copy(src, dst, sem):
        return pltpu.make_async_copy(src, dst, sems.at[sem])

    def lane_tile(t):
        return pl.ds(t * 128, 128)

    def start(copies):
        for c in copies:
            c.start()

    def wait(copies):
        for c in copies:
            c.wait()

    c_ax = [copy(ax_hbm.bitcast(u32).at[:, jp, :], xa.at[jp], jp) for jp in range(8)]
    c_xe = copy(bx_hbm.at[:, pl.ds(0, EARLY), :], xe_raw, sem_xe)
    c_w = [copy(src.bitcast(u32).at[:, j, :], w.at[i * (H // 2) + j], sem_w + (i * (H // 2) + j) // PAIRS)
           for i, src in enumerate((wq_hbm, wk_hbm, wv_hbm)) for j in range(H // 2)]
    c_rest = [copy(wo_hbm.bitcast(u32).at[:, lane_tile(t)], wo.at[t], sem_rest) for t in range(8)]
    c_rest += [copy(m0_hbm, m0, sem_rest), copy(bx_hbm.at[:, pl.ds(EARLY, SEG - EARLY), :], xl, sem_rest)]
    c_aw = [copy(src.at[pl.ds(0, D // 2), :].bitcast(u32).at[:, lane_tile(t)], dst.at[t], sem_rest)
            for src, dst in ((wr_hbm, wra), (wi_hbm, wia)) for t in range(16)]
    c_aw += [copy(wr_hbm.at[pl.ds(D // 2, 1), :], wr_ny, sem_rest),
             copy(wi_hbm.at[pl.ds(D // 2, 1), :], wi_ny, sem_rest)]
    start(c_ax + [c_xe] + c_w[:N_PAIRS // 2])

    row0 = lax.broadcasted_iota(jnp.int32, (8, 128), 0) == 0
    g = lambda i: pltpu.bitcast(g_ref[i], bf16)
    mm = lambda n1, part: pltpu.bitcast(mm_ref[4 * n1 + part], bf16)
    f_re, f_im = _unit_roots(128, 128)
    s_twiddles = _unit_roots(16, S)
    _make_d_matrices(g_ref, f_re, f_im)
    for n1 in range(4):
        _make_s_matrices(mm_ref, n1, f_re, f_im, s_twiddles)
    us = {}
    for arrived, stages in FORWARD_PLAN:
        wait([c_ax[jp] for jp in arrived])
        if 7 in arrived:
            start(c_w[N_PAIRS // 2:] + c_rest)
        for stage in stages.split():
            jp = int(stage[1])
            if stage[0] == "m":
                _forward_matmuls(jp, us.pop(jp), g, mm, fr, fi, row0)
                continue
            us[jp] = _forward_butterflies(jp, xa)
            for n1 in range(max(2 * jp, 4), 2 * jp + 2):
                _make_s_matrices(mm_ref, n1, f_re, f_im, s_twiddles)

    c_xe.wait()
    _make_early_operands(xe_raw, xe)

    def project_early(i, _):
        group = w.at[pl.ds(i * PAIRS, PAIRS)]
        pltpu.make_async_copy(group, group, sems.at[sem_w + i]).wait()

        @pl.when(i == N_PAIRS // PAIRS // 2)
        def _():
            start(c_aw)

        for u in range(PAIRS):
            _project_early_rows(i * PAIRS + u, xe, w, early)
            _repack_head_pair(w, i * PAIRS + u)
        return 0

    lax.fori_loop(0, N_PAIRS // PAIRS, project_early, 0)
    wait(c_rest + c_aw)

    row = lax.broadcasted_iota(jnp.int32, (L, L), 0)
    col = lax.broadcasted_iota(jnp.int32, (L, L), 1)
    mask = (row < M) | (row >= col)

    def segments(with_filter, i, mem):
        for s in [i * UNROLL + u for u in range(UNROLL)]:
            pieces = _filter_two_classes(s, wra, wia, fr, fi, row0) if with_filter else []

            def side_work(fresh):
                if pieces:
                    fr[0, pl.ds(PACE_ROW, 8), :] = fresh
                    fi[0, pl.ds(PACE_ROW, 8), :] = fresh
                    pieces.pop(0)()

            mem = _segment(s, mem, xl, w, wo, early, ob, mask, side_work)
            assert not pieces
        rows = pl.ds(2 * UNROLL * i, 2 * UNROLL)
        pltpu.make_async_copy(ob.at[rows], out_hbm.at[rows, :, pl.ds(D, D)], ob_sem).start()
        return mem

    mem = lax.fori_loop(0, 32 // UNROLL, functools.partial(segments, True), m0[...].astype(f32))

    _filter_nyquist(wr_ny, wi_ny, fr, fi)
    for jp in range(8):
        _inverse(jp, fr, fi, g, mm, ya, row0)
    c_ya = [pltpu.make_async_copy(ya.at[jp], out_hbm.bitcast(u32).at[:, jp, pl.ds(0, D)], ya_sem)
            for jp in range(8)]
    start(c_ya)

    lax.fori_loop(32 // UNROLL, NSEG // UNROLL, functools.partial(segments, False), mem)
    wait(c_ya)
    pltpu.make_async_copy(ob, ob, ob_sem).wait()


def _run(A_x, A_w_r, A_w_i, B_x, B_mem0, B_Wq, B_Wk, B_Wv, B_Wo):
    hbm = pl.BlockSpec(memory_space=pltpu.HBM)
    out = pl.pallas_call(
        _kernel,
        out_shape=jax.ShapeDtypeStruct((S // 16, 16, 2 * D), bf16),
        in_specs=[hbm] * 9,
        out_specs=hbm,
        scratch_shapes=[
            pltpu.VMEM((8, 128, D), u32),
            pltpu.VMEM((16, D // 4, 128), u32),
            pltpu.VMEM((16, D // 4, 128), u32),
            pltpu.VMEM((1, S), bf16),
            pltpu.VMEM((1, S), bf16),
            pltpu.VMEM((11, 64, 128), u32),
            pltpu.VMEM((64, 64, 128), u32),
            pltpu.VMEM((16, PACE_ROW + 8, 128), f32),
            pltpu.VMEM((16, PACE_ROW + 8, 128), f32),
            pltpu.VMEM((8, 128, D), u32),
            pltpu.VMEM((N_PAIRS, D, DH), u32),
            pltpu.VMEM((8, H * DH // 2, 128), u32),
            pltpu.VMEM((NSEG, EARLY, D), bf16),
            pltpu.VMEM((7, 4, NSEG * EARLY // 4, 128), u32),
            pltpu.VMEM((NSEG, SEG - EARLY, D), bf16),
            pltpu.VMEM((M, D), bf16),
            pltpu.VMEM((3 * H, NSEG * EARLY, DH), f32),
            pltpu.VMEM((S // 16, 16, D), bf16),
            pltpu.SemaphoreType.DMA((10 + N_PAIRS // PAIRS,)),
            pltpu.SemaphoreType.DMA(()),
            pltpu.SemaphoreType.DMA(()),
        ],
        compiler_params=pltpu.CompilerParams(vmem_limit_bytes=120 * 1024 * 1024),
        name="gfnet_rmt",
    )(A_x.reshape(S // 16, 16, D), A_w_r.T, A_w_i.T, B_x.reshape(NSEG, SEG, D), B_mem0.reshape(M, D),
      B_Wq, B_Wk, B_Wv, B_Wo.reshape(H * DH, D))
    return out.reshape(1, S, 2 * D)


_run_jit = jax.jit(_run)


def pallas_concat_heads__spectral_gfnet__memory_aug_recurrent_mem_tr__prompt_kernel(
    A_x, A_w_r, A_w_i, B_x, B_mem0, B_Wq, B_Wk, B_Wv, B_Wo, B_seg_len,
):
    assert A_x.shape == (1, S, D) and B_x.shape == (1, S, D) and B_mem0.shape == (1, M, D)
    assert B_Wq.shape == (D, H, DH) and B_Wo.shape == (H, DH, D)
    assert B_seg_len == SEG, "the kernel is built for the problem's segment length"
    return _run_jit(A_x, A_w_r, A_w_i, B_x, B_mem0, B_Wq, B_Wk, B_Wv, B_Wo)
```

```python
import functools

import jax
import jax.numpy as jnp
import numpy as np
from jax import lax
import jax.experimental.pallas as pl
import jax.experimental.pallas.tpu as pltpu

f32, bf16, u32 = jnp.float32, jnp.bfloat16, jnp.uint32

S = 2048
D = 1024
H, DH = 32, 128
M = 8
SEG = 32
L = M + SEG
NSEG = S // SEG
EARLY = 8
GH = 4
NG = H // GH
UNROLL = 2
PAIRS = 6
N_PAIRS = 3 * H // 2

CLASS_PAIRS = ((0, 4), (1, 7), (2, 6), (3, 5))
NYQUIST_ROW = D // 2
PACE_ROW = NYQUIST_ROW + 8
RH = float(np.sqrt(0.5))
LOG2E = float(np.log2(np.e))
LO_MASK, HI_MASK = np.uint32(0xFFFF), np.uint32(0xFFFF0000)

FORWARD_PLAN = (
    ((0,), "b0 m0"),
    ((1,), "b1"),
    ((2,), "m1 b2"),
    ((3, 4), "m2 b3 m3 b4"),
    ((5, 6, 7), "m4 b5 m5 b6 m6 b7 m7"),
)


def _dot(a, b):
    return lax.dot_general(a, b, (((1,), (0,)), ((), ())), preferred_element_type=f32)


def _dot_t(a, b):
    return lax.dot_general(a, b, (((1,), (1,)), ((), ())), preferred_element_type=f32)


def _lo_f32(words):
    return pltpu.bitcast(words << 16, f32)


def _hi_f32(words):
    return pltpu.bitcast(words & HI_MASK, f32)


def _unit_roots(rows, n):
    shape = (rows, 128)
    turns = (lax.broadcasted_iota(jnp.int32, shape, 0) * lax.broadcasted_iota(jnp.int32, shape, 1)) & (n - 1)
    angle = turns.astype(f32) * (-2 * np.pi / n)
    return jnp.cos(angle), jnp.sin(angle)


def _put_bf16(ref, i, val):
    ref[i] = pltpu.bitcast(val.astype(bf16), u32)


def _rotate(re, im, twiddles, i):
    c, s = twiddles[0][i:i + 1], twiddles[1][i:i + 1]
    return re * c - im * s, re * s + im * c


def _make_d_matrices(g_ref, f_re, f_im):
    twiddles = _unit_roots(8, D)
    re, im = f_re[:72] * 2.0 ** -10, f_im[:64] * 2.0 ** -10
    cls = [_rotate(re[:64], im, twiddles, r) for r in range(8)]
    first = lax.broadcasted_iota(jnp.int32, (64, 128), 0) == 0
    _put_bf16(g_ref, 0, jnp.concatenate([cls[0][0], jnp.where(first, re[64:65], cls[0][1])], axis=0))
    _put_bf16(g_ref, 1, jnp.concatenate(cls[4], axis=0))
    for r in (1, 2, 3):
        (c, s), (c_, s_) = cls[r], cls[8 - r]
        _put_bf16(g_ref, 3 * r - 1, jnp.concatenate([c, c_], axis=0))
        _put_bf16(g_ref, 3 * r, jnp.concatenate([c + s, c_ - s_], axis=0))
        _put_bf16(g_ref, 3 * r + 1, jnp.concatenate([s - c, s_ + c_], axis=0))


def _make_s_matrices(mm_ref, n1, f_re, f_im, twiddles):
    parts = []
    for r0 in range(0, 128, 8):
        re, im = _rotate(f_re[r0:r0 + 8], f_im[r0:r0 + 8], twiddles, n1)
        parts.append((re, re + im, im - re, im))
    for i, tile in enumerate(zip(*parts)):
        _put_bf16(mm_ref, 4 * n1 + i, jnp.concatenate(tile, axis=0))


def _forward_butterflies(jp, xa):
    def rows(r0, cvt):
        x = [cvt(xa[jp, pl.ds(r0, 8), pl.ds(t * 128, 128)]) for t in range(8)]
        a = [x[i] + x[i + 4] for i in range(4)]
        b = [x[i] - x[i + 4] for i in range(4)]
        e0, e1 = a[0] + a[2], a[1] + a[3]
        t0, t1 = (b[1] - b[3]) * RH, (b[1] + b[3]) * -RH
        u = [e0 + e1, e0 - e1]
        for p, q in ((b[0] + t0, t1 - b[2]), (a[0] - a[2], a[3] - a[1]), (b[0] - t0, b[2] + t1)):
            u += [p + q, q, p]
        return u

    us = []
    for cvt in (_lo_f32, _hi_f32):
        parts = [rows(r0, cvt) for r0 in range(0, 128, 8)]
        us.append([jnp.concatenate(tile, axis=0).astype(bf16) for tile in zip(*parts)])
    return us


def _forward_matmuls(jp, us, g, mm, fr, fi, row0):
    spectra = []
    for u in us:
        d0, d4 = _dot_t(g(0), u[0]), _dot_t(g(1), u[1])
        nyquist = d0[64:72]
        x = [(jnp.concatenate([d0[:64], d4[:64]], axis=0),
              jnp.concatenate([jnp.where(row0, 0.0, nyquist), d0[72:], d4[64:]], axis=0))]
        for r in (1, 2, 3):
            t1, t2, t3 = [_dot_t(g(3 * r - 1 + i), u[3 * r - 1 + i]) for i in range(3)]
            x.append((t1 - t2, jnp.concatenate([t3[:64] + t1[:64], t3[64:] - t1[64:]], axis=0)))
        spectra.append((nyquist, x))
    for half, (nyquist, x) in enumerate(spectra):
        n1 = 2 * jp + half
        for classes, (re, im) in zip(CLASS_PAIRS, x):
            extra = [nyquist] if classes[0] == 0 else []
            t1 = _dot(jnp.concatenate([re + im] + extra, axis=0), mm(n1, 0))
            t2 = _dot(im, mm(n1, 1))
            t3 = _dot(jnp.concatenate([re] + extra, axis=0), mm(n1, 2))
            for i, c in enumerate(classes):
                rows = slice(64 * i, 64 * i + 64)
                fr[n1, pl.ds(64 * c, 64), :] = t1[rows] - t2[rows]
                fi[n1, pl.ds(64 * c, 64), :] = t1[rows] + t3[rows]
            if extra:
                fr[n1, pl.ds(NYQUIST_ROW, 8), :] = t1[128:]
                fi[n1, pl.ds(NYQUIST_ROW, 8), :] = t1[128:] + t3[128:]


def _fft4(z, sgn):
    a, b, c, d = z
    t0 = (a[0] + c[0], a[1] + c[1])
    t1 = (a[0] - c[0], a[1] - c[1])
    t2 = (b[0] + d[0], b[1] + d[1])
    t3 = (b[0] - d[0], b[1] - d[1])
    o0 = (t0[0] + t2[0], t0[1] + t2[1])
    o2 = (t0[0] - t2[0], t0[1] - t2[1])
    p = (t1[0] + t3[1], t1[1] - t3[0])
    m = (t1[0] - t3[1], t1[1] + t3[0])
    return (o0, p, o2, m) if sgn < 0 else (o0, m, o2, p)


def _twiddle16(v, e, sgn):
    re, im = v
    if e == 0:
        return v
    if e == 4:
        return (im, -re) if sgn < 0 else (-im, re)
    if e == 2:
        return ((re + im) * RH, (im - re) * RH) if sgn < 0 else ((re - im) * RH, (im + re) * RH)
    if e == 6:
        return ((im - re) * RH, (re + im) * -RH) if sgn < 0 else ((re + im) * -RH, (re - im) * RH)
    c, s = float(np.cos(np.pi * e / 8)), float(sgn * np.sin(np.pi * e / 8))
    return (re * c - im * s, re * s + im * c)


def _filter_pieces(r0, weight, fr, fi):
    rows = pl.ds(r0, 8)

    def load(ns):
        return [(fr[n, rows, :], fi[n, rows, :]) for n in ns]

    def store(ns, z):
        for n, (re, im) in zip(ns, z):
            fr[n, rows, :] = re
            fi[n, rows, :] = im

    def outer(a, sgn):
        ns = [a, a + 4, a + 8, a + 12]
        store(ns, _fft4(load(ns), sgn))

    def inner(kl):
        ns = [4 * kl + a for a in range(4)]
        z = _fft4([_twiddle16(v, a * kl, -1) for a, v in enumerate(load(ns))], -1)
        y = []
        for kh, (re, im) in enumerate(z):
            wr, wi = weight(kl + 4 * kh)
            y.append((re * wr - im * wi, re * wi + im * wr))
        store(ns, [_twiddle16(v, a * kl, 1) for a, v in enumerate(_fft4(y, 1))])

    return ([functools.partial(outer, a, -1) for a in range(4)]
            + [functools.partial(inner, kl) for kl in range(4)]
            + [functools.partial(outer, a, 1) for a in range(4)])


def _filter_two_classes(i, wra, wia, fr, fi, row0):
    rho, jb = i // 8, i % 8
    words = pl.ds(rho + 32 * jb, 8, stride=4)
    once = jnp.where(jnp.logical_and(row0, i == 0), 0.5, 1.0)
    even = lambda k: (_lo_f32(wra[k, words, :]) * once, _lo_f32(wia[k, words, :]) * once)
    odd = lambda k: (_hi_f32(wra[k, words, :]), _hi_f32(wia[k, words, :]))
    r0 = rho * 128 + jb * 8
    return (_filter_pieces(pl.multiple_of(r0, 8), even, fr, fi)
            + _filter_pieces(pl.multiple_of(r0 + 64, 8), odd, fr, fi))


def _filter_nyquist(wr_ny, wi_ny, fr, fi):
    wr, wi = wr_ny[...].astype(f32) * 0.5, wi_ny[...].astype(f32) * 0.5
    weight = lambda k: (wr[:, k * 128:(k + 1) * 128], wi[:, k * 128:(k + 1) * 128])
    for piece in _filter_pieces(NYQUIST_ROW, weight, fr, fi):
        piece()


def _inverse(jp, fr, fi, g, mm, ya, row0):
    sign = jnp.where(lax.broadcasted_iota(jnp.int32, (1, 128), 1) < 64, 1.0, -1.0)
    zs = []
    for n1 in (2 * jp, 2 * jp + 1):
        rows = lambda ref, c: ref[n1, pl.ds(64 * c, 64), :]
        z = {}
        for classes in CLASS_PAIRS[1:]:
            br = jnp.concatenate([rows(fr, c) for c in classes], axis=0)
            bi = jnp.concatenate([rows(fi, c) for c in classes], axis=0)
            t1 = _dot_t(mm(n1, 0), (br + bi).astype(bf16))
            z[classes[0]] = (t1 + _dot_t(mm(n1, 2), bi.astype(bf16)), t1 - _dot_t(mm(n1, 1), br.astype(bf16)))
        for c in (4, 0):
            br, bi = rows(fr, c), rows(fi, c)
            b1, b2 = bi, -br
            if c == 0:
                b1 = jnp.concatenate([jnp.where(row0, fr[n1, pl.ds(NYQUIST_ROW, 8), :], b1[:8]), b1[8:]], axis=0)
                b2 = jnp.concatenate([jnp.where(row0, fi[n1, pl.ds(NYQUIST_ROW, 8), :], b2[:8]), b2[8:]], axis=0)
            z[c] = (_dot_t(mm(n1, 0), jnp.concatenate([br, b1], axis=0).astype(bf16))
                    + _dot_t(mm(n1, 3), jnp.concatenate([bi, b2], axis=0).astype(bf16)))
        zs.append(z)
    vs = []
    for z in zs:
        v = []
        for r in (1, 2, 3):
            re, im = z[r]
            t1 = _dot(re + im * sign, g(3 * r - 1))
            v += [t1 + _dot(im, g(3 * r + 1)), t1 - _dot(re, g(3 * r))]
        vs.append(v + [_dot(z[4], g(1)), _dot(z[0], g(0))])
    for r0 in range(0, 128, 8):
        ys = []
        for v in vs:
            p1, q1, p2, q2, p3, q3, v4, v0 = [t[r0:r0 + 8] for t in v]
            e0, e1 = v0 + v4, v0 - v4
            a0, a2, a1, a3 = e0 + p2, e0 - p2, e1 - q2, e1 + q2
            b0, b2 = p1 + p3, q3 - q1
            t0, t1 = p1 - p3, q1 + q3
            b1, b3 = (t0 - t1) * RH, (t0 + t1) * -RH
            ys.append([a0 + b0, a1 + b1, a2 + b2, a3 + b3, a0 - b0, a1 - b1, a2 - b2, a3 - b3])
        for t in range(8):
            lo = pltpu.bitcast(ys[0][t].astype(bf16).astype(f32), u32) >> 16
            hi = pltpu.bitcast(ys[1][t].astype(bf16).astype(f32), u32)
            ya[t, pl.ds(8 * r0 + jp, 8, stride=8), :] = lo | hi


def _repack_head_pair(w, j):
    for r0 in range(0, D, 16):
        even = w[j, pl.ds(r0, 8, stride=2), :]
        odd = w[j, pl.ds(r0 + 1, 8, stride=2), :]
        w[j, pl.ds(r0, 8), :] = (even & LO_MASK) | (odd << 16)
        w[j, pl.ds(r0 + 8, 8), :] = (even >> 16) | (odd & HI_MASK)


def _head_weight(w, j, parity):
    words = w[j].reshape(D // 16, 2, 8, DH)[:, parity].reshape(D // 2, DH)
    return pltpu.bitcast(words, bf16)


def _make_early_operands(xe_raw, xe):
    for i in range(NSEG // 4):
        top, bottom = [jnp.concatenate([xe_raw[s].astype(f32), xe_raw[s + 1].astype(f32)], axis=0)
                       for s in (2 * i, NSEG // 2 + 2 * i)]
        for t in range(4):
            a11, a12, a21, a22 = [half[:, c:c + 128] for half in (top, bottom)
                                  for c in (t * 128, D // 2 + t * 128)]
            for n, val in enumerate((a11 + a22, a21 + a22, a11, a22, a11 + a12, a21 - a11, a12 - a22)):
                xe[n, t, pl.ds(8 * i, 8), :] = pltpu.bitcast(val.astype(bf16), u32)


def _project_early_rows(j, xe, w, early):
    b11, b12 = (lambda r0, cvt=cvt: cvt(w[j, pl.ds(r0, 8), :]) for cvt in (_lo_f32, _hi_f32))
    b21, b22 = (lambda r0, cvt=cvt: cvt(w[j, pl.ds(D // 2 + r0, 8), :]) for cvt in (_lo_f32, _hi_f32))

    def product(n, right):
        total = None
        for t in range(4):
            tile = jnp.concatenate([right(r0) for r0 in range(t * 128, t * 128 + 128, 8)], axis=0)
            part = _dot(pltpu.bitcast(xe[n, t], bf16), tile.astype(bf16))
            total = part if total is None else total + part
        return total

    half = NSEG * EARLY // 2
    m1 = product(0, lambda r: b11(r) + b22(r))
    m4 = product(3, lambda r: b21(r) - b11(r))
    c11 = m1 + m4 + product(6, lambda r: b21(r) + b22(r))
    m5 = product(4, b22)
    early[2 * j, pl.ds(0, half), :] = c11 - m5
    m3 = product(2, lambda r: b12(r) - b22(r))
    early[2 * j + 1, pl.ds(0, half), :] = m3 + m5
    m2 = product(1, b11)
    early[2 * j, pl.ds(half, half), :] = m2 + m4
    early[2 * j + 1, pl.ds(half, half), :] = m1 + m3 - m2 + product(5, lambda r: b11(r) + b12(r))


def _segment(s, mem, xl, w, wo, early, ob, mask, side_work):
    hh = jnp.concatenate([mem, xl[s].astype(f32)], axis=0).astype(bf16)
    early_rows = pl.ds(pl.multiple_of(s * EARLY, EARLY), EARLY)
    q, k, v, p, o = {}, {}, {}, {}, {}
    acc = [None] * 8
    heads = lambda grp: range(grp * GH, (grp + 1) * GH)

    def project_one(i, h):
        y = _dot(hh, _head_weight(w, i * (H // 2) + h // 2, h % 2))
        return jnp.concatenate([y[:M], early[i * H + h, early_rows, :], y[M:]], axis=0)

    def project(grp):
        for h in heads(grp):
            q[h] = project_one(0, h)
            k[h] = project_one(1, h).astype(bf16)
            v[h] = project_one(2, h).astype(bf16)

    def softmax(grp):
        for h in heads(grp):
            scores = jnp.where(mask, _dot_t(q.pop(h), k.pop(h)) * (DH ** -0.5 * LOG2E), -1e9 * LOG2E)
            e = jnp.exp2(scores - jnp.max(scores, axis=1, keepdims=True))
            total = jnp.sum(e, axis=1, keepdims=True)
            r = pltpu.reciprocal(total, approx=True)
            p[h] = e * (r * (2.0 - total * r))

    def mix(grp):
        for h in heads(grp):
            o[h] = _dot(p.pop(h), v.pop(h))

    def out_project(grp, tiles=range(8)):
        og = jnp.concatenate([o[h] for h in heads(grp)], axis=1)
        for j in tiles:
            t = _dot(og, pltpu.bitcast(wo[j, pl.ds(grp * GH * DH // 2, GH * DH // 2), :], bf16))
            acc[j] = t if acc[j] is None else acc[j] + t
            if j < 4:
                side_work(t[:8])

    for t in range(NG):
        project(t)
        if t >= 1:
            softmax(t - 1)
        if t >= 2:
            mix(t - 2)
        if t >= 4:
            out_project(t - 4)
    out_project(NG - 4, range(4))
    softmax(NG - 1)
    mix(NG - 2)
    out_project(NG - 4, range(4, 8))
    out_project(NG - 3)
    mix(NG - 1)
    out_project(NG - 2)
    out_project(NG - 1)

    res = jnp.concatenate(acc, axis=1)
    ob[pl.ds(pl.multiple_of(s * SEG, SEG), SEG), :] = res[M:].astype(bf16)
    return res[:M].astype(bf16).astype(f32)


def _kernel(ax_hbm, wr_hbm, wi_hbm, bx_hbm, m0_hbm, wq_hbm, wk_hbm, wv_hbm, wo_hbm, out_hbm,
            xa, wra, wia, wr_ny, wi_ny, g_ref, mm_ref, fr, fi, ya,
            w, wo, xe_raw, xe, xl, m0, early, ob, sems, ya_sem, ob_sem):
    sem_xe, sem_rest, sem_w = 8, 9, 10

    def copy(src, dst, sem):
        return pltpu.make_async_copy(src, dst, sems.at[sem])

    def lane_tile(t):
        return pl.ds(t * 128, 128)

    def start(copies):
        for c in copies:
            c.start()

    def wait(copies):
        for c in copies:
            c.wait()

    c_ax = [copy(ax_hbm.bitcast(u32).at[:, jp, :], xa.at[jp], jp) for jp in range(8)]
    c_xe = copy(bx_hbm.at[:, pl.ds(0, EARLY), :], xe_raw, sem_xe)
    c_w = [copy(src.bitcast(u32).at[:, j, :], w.at[i * (H // 2) + j], sem_w + (i * (H // 2) + j) // PAIRS)
           for i, src in enumerate((wq_hbm, wk_hbm, wv_hbm)) for j in range(H // 2)]
    c_rest = [copy(wo_hbm.bitcast(u32).at[:, lane_tile(t)], wo.at[t], sem_rest) for t in range(8)]
    c_rest += [copy(m0_hbm, m0, sem_rest), copy(bx_hbm.at[:, pl.ds(EARLY, SEG - EARLY), :], xl, sem_rest)]
    c_aw = [copy(src.at[pl.ds(0, D // 2), :].bitcast(u32).at[:, lane_tile(t)], dst.at[t], sem_rest)
            for src, dst in ((wr_hbm, wra), (wi_hbm, wia)) for t in range(16)]
    c_aw += [copy(wr_hbm.at[pl.ds(D // 2, 1), :], wr_ny, sem_rest),
             copy(wi_hbm.at[pl.ds(D // 2, 1), :], wi_ny, sem_rest)]
    start(c_ax + [c_xe] + c_w[:N_PAIRS // 2])

    row0 = lax.broadcasted_iota(jnp.int32, (8, 128), 0) == 0
    g = lambda i: pltpu.bitcast(g_ref[i], bf16)
    mm = lambda n1, part: pltpu.bitcast(mm_ref[4 * n1 + part], bf16)
    f_re, f_im = _unit_roots(128, 128)
    s_twiddles = _unit_roots(16, S)
    _make_d_matrices(g_ref, f_re, f_im)
    for n1 in range(4):
        _make_s_matrices(mm_ref, n1, f_re, f_im, s_twiddles)
    us = {}
    for arrived, stages in FORWARD_PLAN:
        wait([c_ax[jp] for jp in arrived])
        if 7 in arrived:
            start(c_w[N_PAIRS // 2:] + c_rest)
        for stage in stages.split():
            jp = int(stage[1])
            if stage[0] == "m":
                _forward_matmuls(jp, us.pop(jp), g, mm, fr, fi, row0)
                continue
            us[jp] = _forward_butterflies(jp, xa)
            for n1 in range(max(2 * jp, 4), 2 * jp + 2):
                _make_s_matrices(mm_ref, n1, f_re, f_im, s_twiddles)

    c_xe.wait()
    _make_early_operands(xe_raw, xe)

    def project_early(i, _):
        group = w.at[pl.ds(i * PAIRS, PAIRS)]
        pltpu.make_async_copy(group, group, sems.at[sem_w + i]).wait()

        @pl.when(i == N_PAIRS // PAIRS // 2)
        def _():
            start(c_aw)

        for u in range(PAIRS):
            _project_early_rows(i * PAIRS + u, xe, w, early)
            _repack_head_pair(w, i * PAIRS + u)
        return 0

    lax.fori_loop(0, N_PAIRS // PAIRS, project_early, 0)
    wait(c_rest + c_aw)

    row = lax.broadcasted_iota(jnp.int32, (L, L), 0)
    col = lax.broadcasted_iota(jnp.int32, (L, L), 1)
    mask = (row < M) | (row >= col)

    def segments(with_filter, i, mem):
        for s in [i * UNROLL + u for u in range(UNROLL)]:
            pieces = _filter_two_classes(s, wra, wia, fr, fi, row0) if with_filter else []

            def side_work(fresh):
                if pieces:
                    fr[0, pl.ds(PACE_ROW, 8), :] = fresh
                    fi[0, pl.ds(PACE_ROW, 8), :] = fresh
                    pieces.pop(0)()

            mem = _segment(s, mem, xl, w, wo, early, ob, mask, side_work)
            assert not pieces
        rows = pl.ds(pl.multiple_of(i * UNROLL * SEG, UNROLL * SEG), UNROLL * SEG)
        pltpu.make_async_copy(ob.at[rows], out_hbm.at[rows, pl.ds(D, D)], ob_sem).start()
        return mem

    mem = lax.fori_loop(0, 32 // UNROLL, functools.partial(segments, True), m0[...].astype(f32))

    _filter_nyquist(wr_ny, wi_ny, fr, fi)
    for jp in range(8):
        _inverse(jp, fr, fi, g, mm, ya, row0)
    c_ya = [pltpu.make_async_copy(ya.bitcast(bf16).at[t], out_hbm.at[:, lane_tile(t)], ya_sem)
            for t in range(8)]
    start(c_ya)

    lax.fori_loop(32 // UNROLL, NSEG // UNROLL, functools.partial(segments, False), mem)
    wait(c_ya)
    pltpu.make_async_copy(ob, ob, ob_sem).wait()


def _run(A_x, A_w_r, A_w_i, B_x, B_mem0, B_Wq, B_Wk, B_Wv, B_Wo):
    hbm = pl.BlockSpec(memory_space=pltpu.HBM)
    out = pl.pallas_call(
        _kernel,
        out_shape=jax.ShapeDtypeStruct((S, 2 * D), bf16),
        in_specs=[hbm] * 9,
        out_specs=hbm,
        scratch_shapes=[
            pltpu.VMEM((8, 128, D), u32),
            pltpu.VMEM((16, D // 4, 128), u32),
            pltpu.VMEM((16, D // 4, 128), u32),
            pltpu.VMEM((1, S), bf16),
            pltpu.VMEM((1, S), bf16),
            pltpu.VMEM((11, 64, 128), u32),
            pltpu.VMEM((64, 64, 128), u32),
            pltpu.VMEM((16, PACE_ROW + 8, 128), f32),
            pltpu.VMEM((16, PACE_ROW + 8, 128), f32),
            pltpu.VMEM((8, S // 2, 128), u32),
            pltpu.VMEM((N_PAIRS, D, DH), u32),
            pltpu.VMEM((8, H * DH // 2, 128), u32),
            pltpu.VMEM((NSEG, EARLY, D), bf16),
            pltpu.VMEM((7, 4, NSEG * EARLY // 4, 128), u32),
            pltpu.VMEM((NSEG, SEG - EARLY, D), bf16),
            pltpu.VMEM((M, D), bf16),
            pltpu.VMEM((3 * H, NSEG * EARLY, DH), f32),
            pltpu.VMEM((S, D), bf16),
            pltpu.SemaphoreType.DMA((10 + N_PAIRS // PAIRS,)),
            pltpu.SemaphoreType.DMA(()),
            pltpu.SemaphoreType.DMA(()),
        ],
        compiler_params=pltpu.CompilerParams(vmem_limit_bytes=100 * 1024 * 1024),
        name="gfnet_rmt",
    )(A_x.reshape(S // 16, 16, D), A_w_r.T, A_w_i.T, B_x.reshape(NSEG, SEG, D), B_mem0.reshape(M, D),
      B_Wq, B_Wk, B_Wv, B_Wo.reshape(H * DH, D))
    return out.reshape(1, S, 2 * D)


_run_jit = jax.jit(_run)


def pallas_concat_heads__spectral_gfnet__memory_aug_recurrent_mem_tr__prompt_kernel(
    A_x, A_w_r, A_w_i, B_x, B_mem0, B_Wq, B_Wk, B_Wv, B_Wo, B_seg_len,
):
    assert A_x.shape == (1, S, D) and B_x.shape == (1, S, D) and B_mem0.shape == (1, M, D)
    assert B_Wq.shape == (D, H, DH) and B_Wo.shape == (H, DH, D)
    assert B_seg_len == SEG, "the kernel is built for the problem's segment length"
    return _run_jit(A_x, A_w_r, A_w_i, B_x, B_mem0, B_Wq, B_Wk, B_Wv, B_Wo)
```
